```python
import jax
import jax.numpy as jnp

def _softmax(x, axis=-1):
    return jax.nn.softmax(x, axis=axis)

def _gelu(x):
    return jax.nn.gelu(x, approximate=True)

def _silu(x):
    return jax.nn.silu(x)

def _sigmoid(x):
    return jax.nn.sigmoid(x)

def _layernorm(x, axis=-1, eps=1e-05):
    m = jnp.mean(x, axis=axis, keepdims=True)
    v = jnp.var(x, axis=axis, keepdims=True)
    return (x - m) / jnp.sqrt(v + eps)

def _scatter_add(tgt, idx, src, axis=0):
    return tgt.at[idx].add(src)

def _segment_sum(src, seg, n):
    return jax.ops.segment_sum(src, seg, n)

class _Rng:

    def __init__(self, key):
        self._k = key

    def _next(self):
        self._k, sub = jax.random.split(self._k)
        return sub

    def normal(self, shape):
        return jax.random.normal(self._next(), shape, dtype=jnp.bfloat16)

    def randint(self, lo, hi, shape):
        return jax.random.randint(self._next(), shape, lo, hi, dtype=jnp.int32)

    def uniform(self, shape, lo=0.0, hi=1.0):
        return jax.random.uniform(self._next(), shape, jnp.bfloat16, lo, hi)

    def permutation(self, n):
        return jax.random.permutation(self._next(), n)
kernel_name = 'adaLN_cond__sliding_block_cached__mixer_channel_mlp__decode'

def setup_inputs():
    _rng = _Rng(jax.random.key(int.from_bytes(__import__("os").urandom(4), "little")))
    _w = lambda a: (lambda t: t.astype(jnp.bfloat16) if jnp.issubdtype(t.dtype, jnp.floating) else t)(jnp.asarray(a))

    def _A_setup():
        B, Sq, D = (8, 1, 640)
        Hq, Hkv, Sk, Dh = (32, 32, 4096, 192)
        assert Hq % Hkv == 0, (Hq, Hkv)
        return {'x': _w((lambda *s: _rng.normal(s) * 0.05)(B, Sq, D)), 'k_cache': _w((lambda *s: _rng.normal(s) * 0.05)(B, Hkv, Sk, Dh)), 'v_cache': _w((lambda *s: _rng.normal(s) * 0.05)(B, Hkv, Sk, Dh)), 'wq': _w((lambda *s: _rng.normal(s) * 0.05)(D, Hq * Dh) * D ** (-0.5)), 'wo': _w((lambda *s: _rng.normal(s) * 0.05)(Hq * Dh, D) * (Hq * Dh) ** (-0.5))}
    _A_in = _A_setup()

    def _B_setup():
        B, S, D, F = (8, 1, 640, 1536)
        return {'x': _w((lambda *s: _rng.normal(s) * 0.05)(B, S, D)), 'w1': _w((lambda *s: _rng.normal(s) * 0.05)(D, F) * D ** (-0.5)), 'b1': _w((lambda *s: _rng.normal(s) * 0.05)(F)), 'w2': _w((lambda *s: _rng.normal(s) * 0.05)(F, D) * F ** (-0.5)), 'b2': _w((lambda *s: _rng.normal(s) * 0.05)(D))}
    _B_in = _B_setup()
    return {'A_x': _A_in['x'], 'A_k_cache': _A_in['k_cache'], 'A_v_cache': _A_in['v_cache'], 'A_wq': _A_in['wq'], 'A_wo': _A_in['wo'], 'B_x': _B_in['x'], 'B_w1': _B_in['w1'], 'B_b1': _B_in['b1'], 'B_w2': _B_in['w2'], 'B_b2': _B_in['b2'], 'c': _w((lambda *s: _rng.normal(s) * 0.05)(8, 640)), 'w_mod': _w((lambda *s: _rng.normal(s) * 0.05)(640, 6 * 640) * 640 ** (-0.5))}

def reference(A_x, A_k_cache, A_v_cache, A_wq, A_wo, B_x, B_w1, B_b1, B_w2, B_b2, c, w_mod):

    def _A_ref(x, k_cache, v_cache, wq, wo):
        B, Sq, D = x.shape
        Hq, Dh = (32, 192)
        Hkv, Sk = (k_cache.shape[1], k_cache.shape[2])
        W = min(4096, max(256, Sk // 4))
        rep = Hq // Hkv
        q = (lambda x, *d: x.transpose(*d))((x @ wq).reshape(B, Sq, Hq, Dh), 0, 2, 1, 3)
        k = jnp.repeat(k_cache[:, :, Sk - W:, :], rep, axis=1)
        v = jnp.repeat(v_cache[:, :, Sk - W:, :], rep, axis=1)
        scores = jnp.einsum('bhqd,bhkd->bhqk', q, k) * Dh ** (-0.5)
        p = _softmax(scores, axis=-1)
        o = jnp.einsum('bhqk,bhkd->bhqd', p, v)
        return (lambda x, *d: x.transpose(*d))(o, 0, 2, 1, 3).reshape(B, Sq, Hq * Dh) @ wo

    def _B_ref(x, w1, b1, w2, b2):
        y = _layernorm(x, axis=-1)
        h = _gelu(jnp.einsum('bsd,df->bsf', y, w1) + b1)
        return jnp.einsum('bsf,fd->bsd', h, w2) + b2
    x = A_x
    mod = (_silu(c) @ w_mod).reshape(c.shape[0], 6, 1, -1)
    sa, ca, ga, sb, cb, gb = (mod[:, 0].copy(), mod[:, 1].copy(), mod[:, 2].copy(), mod[:, 3].copy(), mod[:, 4].copy(), mod[:, 5].copy())
    h = _layernorm(x, axis=-1) * (1 + ca) + sa
    x = x + ga * _A_ref(h, A_k_cache, A_v_cache, A_wq, A_wo)
    h = _layernorm(x, axis=-1) * (1 + cb) + sb
    x = x + gb * _B_ref(h, B_w1, B_b1, B_w2, B_b2)
    return x
```

```python
import jax
import jax.numpy as jnp
import jax.experimental.pallas as pl
import jax.experimental.pallas.tpu as pltpu

_EPS = 1e-05
_HG = 8
_NSLOTS = 4


def _layernorm(x):
    m = jnp.mean(x, axis=-1, keepdims=True)
    d = x - m
    v = jnp.mean(d * d, axis=-1, keepdims=True)
    return d / jnp.sqrt(v + _EPS)


def _dot(a, b):
    return jnp.dot(a, b, preferred_element_type=jnp.float32)


@jax.jit
def pallas_adaLN_cond__sliding_block_cached__mixer_channel_mlp__decode_kernel(
    A_x: jax.Array,
    A_k_cache: jax.Array,
    A_v_cache: jax.Array,
    A_wq: jax.Array,
    A_wo: jax.Array,
    B_x: jax.Array,
    B_w1: jax.Array,
    B_b1: jax.Array,
    B_w2: jax.Array,
    B_b2: jax.Array,
    c: jax.Array,
    w_mod: jax.Array,
):
    B, Sq, D = A_x.shape
    _, H, Sk, Dh = A_k_cache.shape
    assert Sq == 1
    F = B_w1.shape[1]
    W = min(4096, max(256, Sk // 4))
    HD = H * Dh
    rows = _HG * Dh
    nj = H // _HG
    nsteps = B * nj
    scale = Dh ** -0.5
    f32, bf16 = jnp.float32, jnp.bfloat16

    def kernel(x_hbm, k_hbm, v_hbm, wq_hbm, wo_hbm, w1_hbm, b1_hbm, w2_hbm, b2_hbm,
               c_hbm, wm_hbm, out_ref,
               x_v, c_v, b1_v, b2_v, wm_v, wq_v, wo_v, w1_v, w2_v,
               kbuf, vbuf, q_s, o_s, kv_sem, w_sem):
        def k_copy(i, slot):
            return pltpu.make_async_copy(
                k_hbm.at[pl.ds(i * rows, rows), pl.ds(Sk - W, W)], kbuf.at[slot],
                kv_sem.at[0, slot])

        def v_copy(i, slot):
            return pltpu.make_async_copy(
                v_hbm.at[pl.ds(i * rows, rows), pl.ds(Sk - W, W)], vbuf.at[slot],
                kv_sem.at[1, slot])

        c_cp = pltpu.make_async_copy(c_hbm, c_v, w_sem.at[0])
        x_cp = pltpu.make_async_copy(x_hbm, x_v, w_sem.at[1])
        b1_cp = pltpu.make_async_copy(b1_hbm, b1_v, w_sem.at[2])
        b2_cp = pltpu.make_async_copy(b2_hbm, b2_v, w_sem.at[3])
        wma_cp = pltpu.make_async_copy(wm_hbm.at[:, pl.ds(0, 2 * D)],
                                       wm_v.at[:, pl.ds(0, 2 * D)], w_sem.at[4])
        wmb_cp = pltpu.make_async_copy(wm_hbm.at[:, pl.ds(2 * D, 4 * D)],
                                       wm_v.at[:, pl.ds(2 * D, 4 * D)], w_sem.at[5])
        w1_cp = pltpu.make_async_copy(w1_hbm, w1_v, w_sem.at[6])
        w2_cp = pltpu.make_async_copy(w2_hbm, w2_v, w_sem.at[7])
        wq_cp = [pltpu.make_async_copy(wq_hbm.at[:, pl.ds(j * rows, rows)], wq_v.at[j],
                                       w_sem.at[8 + j]) for j in range(nj)]
        wo_cp = [pltpu.make_async_copy(wo_hbm.at[pl.ds(j * rows, rows), :], wo_v.at[j],
                                       w_sem.at[8 + nj + j]) for j in range(nj)]

        c_cp.start()
        x_cp.start()
        wma_cp.start()
        for cp in wq_cp:
            cp.start()
        for i in range(_NSLOTS):
            k_copy(i, i).start()
            v_copy(i, i).start()
        b1_cp.start()
        b2_cp.start()

        c_cp.wait()
        x_cp.wait()
        sc = jax.nn.silu(c_v[...].astype(f32)).astype(bf16)
        x = x_v[...].astype(f32)
        ln_x = _layernorm(x)
        wma_cp.wait()
        mod_a = _dot(sc, wm_v[:, 0:2 * D])
        h = (ln_x * (1.0 + mod_a[:, D:2 * D]) + mod_a[:, 0:D]).astype(bf16)
        for j in range(nj):
            wq_cp[j].wait()
            q_s[j] = _dot(h, wq_v[j])

        row_id = jax.lax.broadcasted_iota(jnp.int32, (_HG, rows), 0)
        col_id = jax.lax.broadcasted_iota(jnp.int32, (_HG, rows), 1)
        diag = jnp.logical_and(col_id >= row_id * Dh, col_id < (row_id + 1) * Dh)

        def step(i, carry):
            slot = i % _NSLOTS
            b = i // nj
            j = i % nj
            qrow = q_s[j, pl.ds(b, 1), :]
            qbd = jnp.where(diag, jnp.broadcast_to(qrow, (_HG, rows)), 0.0).astype(bf16)
            k_copy(i, slot).wait()
            s = _dot(qbd, kbuf[slot]) * scale
            m = jnp.max(s, axis=-1, keepdims=True)
            p = jnp.exp(s - m)
            l = jnp.sum(p, axis=-1, keepdims=True)
            p = (p / l).astype(bf16)
            v_copy(i, slot).wait()
            o = jax.lax.dot_general(p, vbuf[slot], (((1,), (1,)), ((), ())),
                                    preferred_element_type=f32)
            o_s[j, pl.ds(b, 1), :] = jnp.sum(jnp.where(diag, o, 0.0), axis=0, keepdims=True)

            @pl.when(i + _NSLOTS < nsteps)
            def _():
                k_copy(i + _NSLOTS, slot).start()
                v_copy(i + _NSLOTS, slot).start()

            @pl.when(i + _NSLOTS == nsteps - 1)
            def _():
                for cp in wo_cp:
                    cp.start()
                wmb_cp.start()
                w1_cp.start()
                w2_cp.start()

            return carry

        jax.lax.fori_loop(0, nsteps, step, 0)

        attn = jnp.zeros((B, D), f32)
        for j in range(nj):
            wo_cp[j].wait()
            attn = attn + _dot(o_s[j].astype(bf16), wo_v[j])
        wmb_cp.wait()
        mod_b = _dot(sc, wm_v[:, 2 * D:6 * D])
        ga, sb = mod_b[:, 0:D], mod_b[:, D:2 * D]
        cb, gb = mod_b[:, 2 * D:3 * D], mod_b[:, 3 * D:4 * D]
        x1 = x + ga * attn
        h2 = _layernorm(x1) * (1.0 + cb) + sb
        y = _layernorm(h2).astype(bf16)
        b1_cp.wait()
        b2_cp.wait()
        w1_cp.wait()
        u = _dot(y, w1_v[...]) + b1_v[...].astype(f32).reshape(1, F)
        u = jax.nn.gelu(u, approximate=True).astype(bf16)
        w2_cp.wait()
        mlp = _dot(u, w2_v[...]) + b2_v[...].astype(f32).reshape(1, D)
        out_ref[...] = (x1 + gb * mlp).astype(out_ref.dtype)

    kt = jnp.swapaxes(A_k_cache, 2, 3).reshape(B * HD, Sk)
    vt = jnp.swapaxes(A_v_cache, 2, 3).reshape(B * HD, Sk)
    x2 = A_x.reshape(B, D)

    any_spec = pl.BlockSpec(memory_space=pl.ANY)
    out = pl.pallas_call(
        kernel,
        out_shape=jax.ShapeDtypeStruct((B, D), A_x.dtype),
        in_specs=[any_spec] * 11,
        out_specs=pl.BlockSpec(memory_space=pltpu.VMEM),
        scratch_shapes=[
            pltpu.VMEM((B, D), bf16),
            pltpu.VMEM((B, D), bf16),
            pltpu.VMEM((F,), bf16),
            pltpu.VMEM((D,), bf16),
            pltpu.VMEM((D, 6 * D), bf16),
            pltpu.VMEM((nj, D, rows), bf16),
            pltpu.VMEM((nj, rows, D), bf16),
            pltpu.VMEM((D, F), bf16),
            pltpu.VMEM((F, D), bf16),
            pltpu.VMEM((_NSLOTS, rows, W), bf16),
            pltpu.VMEM((_NSLOTS, rows, W), bf16),
            pltpu.VMEM((nj, B, rows), f32),
            pltpu.VMEM((nj, B, rows), f32),
            pltpu.SemaphoreType.DMA((2, _NSLOTS)),
            pltpu.SemaphoreType.DMA((8 + 2 * nj,)),
        ],
        compiler_params=pltpu.CompilerParams(vmem_limit_bytes=100 * 1024 * 1024),
    )(x2, kt, vt, A_wq, A_wo, B_w1, B_b1, B_w2, B_b2, c, w_mod)
    return out.reshape(B, Sq, D)
```

```python
import jax
import jax.numpy as jnp
import jax.experimental.pallas as pl
import jax.experimental.pallas.tpu as pltpu

_EPS = 1e-05
_HG = 8
_NSLOTS = 3
_STRIPS = (256, 768)
_WO_CHUNKS = 4
_W2_CHUNKS = (1024, 384, 128)


def _layernorm(x):
    m = jnp.mean(x, axis=-1, keepdims=True)
    d = x - m
    v = jnp.mean(d * d, axis=-1, keepdims=True)
    return d / jnp.sqrt(v + _EPS)


def _dot(a, b):
    return jnp.dot(a, b, preferred_element_type=jnp.float32)


def _offsets(sizes):
    return [sum(sizes[:i]) for i in range(len(sizes))]


@jax.jit
def pallas_adaLN_cond__sliding_block_cached__mixer_channel_mlp__decode_kernel(
    A_x: jax.Array,
    A_k_cache: jax.Array,
    A_v_cache: jax.Array,
    A_wq: jax.Array,
    A_wo: jax.Array,
    B_x: jax.Array,
    B_w1: jax.Array,
    B_b1: jax.Array,
    B_w2: jax.Array,
    B_b2: jax.Array,
    c: jax.Array,
    w_mod: jax.Array,
):
    del B_x
    B, Sq, D = A_x.shape
    _, H, Sk, Dh = A_k_cache.shape
    F = B_w1.shape[1]
    W = min(4096, max(256, Sk // 4))
    HD = H * Dh
    assert Sq == 1 and A_wq.shape == (D, HD) and H % _HG == 0
    assert sum(_STRIPS) == W and sum(_W2_CHUNKS) == F and HD % _WO_CHUNKS == 0
    rows = _HG * Dh
    nj = H // _HG
    nsteps = B * nj
    scale = Dh ** -0.5
    f32, bf16 = jnp.float32, jnp.bfloat16
    ns = len(_STRIPS)
    strip_off = _offsets(_STRIPS)
    w2_off = _offsets(_W2_CHUNKS)
    wo_rows = HD // _WO_CHUNKS
    n_kv_sems = 2 * _NSLOTS * ns
    n_sems = n_kv_sems + 7 + _WO_CHUNKS + len(_W2_CHUNKS)

    def kernel(x_hbm, k_hbm, v_hbm, wq_hbm, wo_hbm, w1_hbm, b1_hbm, w2_hbm, b2_hbm,
               c_hbm, wm_hbm, out_ref,
               x_v, c_v, b1_v, b2_v, wm_v, wq_v, wo_v, w1_v, w2_v,
               kbuf, vbuf, q_s, o_s, sem):
        def kv_copies(a, i, slot):
            src, buf = ((k_hbm, kbuf), (v_hbm, vbuf))[a]
            return [
                pltpu.make_async_copy(
                    src.at[pl.ds(i * rows, rows), pl.ds(Sk - W + o, n)],
                    buf.at[slot, :, pl.ds(o, n)],
                    sem.at[(a * _NSLOTS + slot) * ns + s])
                for s, (o, n) in enumerate(zip(strip_off, _STRIPS))]

        def kv_start(i, slot):
            for a in range(2):
                for cp in kv_copies(a, i, slot):
                    cp.start()

        free_sems = iter(range(n_kv_sems, n_sems))

        def copy(src, dst):
            return pltpu.make_async_copy(src, dst, sem.at[next(free_sems)])

        def row_copy(src, dst, o, n):
            return copy(src.at[pl.ds(o, n), :], dst.at[pl.ds(o, n), :])

        c_cp = copy(c_hbm, c_v)
        x_cp = copy(x_hbm, x_v)
        b1_cp = copy(b1_hbm, b1_v)
        b2_cp = copy(b2_hbm, b2_v)
        wm_cp = copy(wm_hbm, wm_v)
        wq_cp = copy(wq_hbm, wq_v)
        w1_cp = copy(w1_hbm, w1_v)
        wo_cp = [row_copy(wo_hbm, wo_v, j * wo_rows, wo_rows) for j in range(_WO_CHUNKS)]
        w2_cp = [row_copy(w2_hbm, w2_v, o, n) for o, n in zip(w2_off, _W2_CHUNKS)]

        for cp in (wm_cp, c_cp, x_cp, wq_cp, b1_cp, b2_cp):
            cp.start()
        for i in range(_NSLOTS):
            kv_start(i, i)

        wm_cp.wait()
        c_cp.wait()
        x_cp.wait()
        x = x_v[...].astype(f32)
        mod = _dot(jax.nn.silu(c_v[...].astype(f32)).astype(bf16), wm_v[...])
        sa, ca, ga, sb, cb, gb = (mod[:, t * D:(t + 1) * D] for t in range(6))
        h = (_layernorm(x) * (1.0 + ca) + sa).astype(bf16)
        wq_cp.wait()
        for j in range(nj):
            q_s[j] = _dot(h, wq_v[:, j * rows:(j + 1) * rows])

        row_id = jax.lax.broadcasted_iota(jnp.int32, (_HG, rows), 0)
        col_id = jax.lax.broadcasted_iota(jnp.int32, (_HG, rows), 1)
        diag = jnp.logical_and(col_id >= row_id * Dh, col_id < (row_id + 1) * Dh)

        def step(i, carry):
            slot = i % _NSLOTS
            b = i // nj
            j = i % nj
            qrow = q_s[j, pl.ds(b, 1), :]
            qbd = jnp.where(diag, jnp.broadcast_to(qrow, (_HG, rows)), 0.0).astype(bf16)
            for cp in kv_copies(0, i, slot):
                cp.wait()
            s = _dot(qbd, kbuf[slot]) * scale
            p = jnp.exp(s - jnp.max(s, axis=-1, keepdims=True))
            p = (p / jnp.sum(p, axis=-1, keepdims=True)).astype(bf16)
            for cp in kv_copies(1, i, slot):
                cp.wait()
            o = jax.lax.dot_general(p, vbuf[slot], (((1,), (1,)), ((), ())),
                                    preferred_element_type=f32)
            o_s[j, pl.ds(b, 1), :] = jnp.sum(jnp.where(diag, o, 0.0), axis=0, keepdims=True)

            @pl.when(i + _NSLOTS < nsteps)
            def _():
                kv_start(i + _NSLOTS, slot)

            @pl.when(i + _NSLOTS == nsteps - 1)
            def _():
                for cp in (*wo_cp, w1_cp, *w2_cp):
                    cp.start()

            return carry

        jax.lax.fori_loop(0, nsteps, step, 0)

        o_all = jnp.concatenate([o_s[j] for j in range(nj)], axis=1).astype(bf16)
        attn = jnp.zeros((B, D), f32)
        for j in range(_WO_CHUNKS):
            wo_cp[j].wait()
            lo, hi = j * wo_rows, (j + 1) * wo_rows
            attn = attn + _dot(o_all[:, lo:hi], wo_v[lo:hi, :])
        x1 = x + ga * attn
        h2 = _layernorm(x1) * (1.0 + cb) + sb
        y = _layernorm(h2).astype(bf16)
        b1_cp.wait()
        b2_cp.wait()
        w1_cp.wait()
        u = _dot(y, w1_v[...]) + b1_v[...].astype(f32).reshape(1, F)
        u = jax.nn.gelu(u, approximate=True).astype(bf16)
        mlp = b2_v[...].astype(f32).reshape(1, D)
        for cp, o, n in zip(w2_cp, w2_off, _W2_CHUNKS):
            cp.wait()
            mlp = mlp + _dot(u[:, o:o + n], w2_v[o:o + n, :])
        out_ref[...] = (x1 + gb * mlp).astype(out_ref.dtype)

    kt = jnp.swapaxes(A_k_cache, 2, 3).reshape(B * HD, Sk)
    vt = jnp.swapaxes(A_v_cache, 2, 3).reshape(B * HD, Sk)

    out = pl.pallas_call(
        kernel,
        out_shape=jax.ShapeDtypeStruct((B, D), A_x.dtype),
        in_specs=[pl.BlockSpec(memory_space=pl.ANY)] * 11,
        out_specs=pl.BlockSpec(memory_space=pltpu.VMEM),
        scratch_shapes=[
            pltpu.VMEM((B, D), bf16),
            pltpu.VMEM((B, D), bf16),
            pltpu.VMEM((F,), bf16),
            pltpu.VMEM((D,), bf16),
            pltpu.VMEM((D, 6 * D), bf16),
            pltpu.VMEM((D, HD), bf16),
            pltpu.VMEM((HD, D), bf16),
            pltpu.VMEM((D, F), bf16),
            pltpu.VMEM((F, D), bf16),
            pltpu.VMEM((_NSLOTS, rows, W), bf16),
            pltpu.VMEM((_NSLOTS, rows, W), bf16),
            pltpu.VMEM((nj, B, rows), f32),
            pltpu.VMEM((nj, B, rows), f32),
            pltpu.SemaphoreType.DMA((n_sems,)),
        ],
        compiler_params=pltpu.CompilerParams(
            vmem_limit_bytes=96 * 1024 * 1024,
            disable_bounds_checks=True,
            disable_semaphore_checks=True,
        ),
    )(A_x.reshape(B, D), kt, vt, A_wq, A_wo, B_w1, B_b1, B_w2, B_b2, c, w_mod)
    return out.reshape(B, Sq, D)
```

```python
import jax
import jax.numpy as jnp
import jax.experimental.pallas as pl
import jax.experimental.pallas.tpu as pltpu

_EPS = 1e-05
_HG = 16
_MAJ = 64
_WO_CHUNKS = 4
_W2_CHUNKS = (1024, 384, 128)


def _layernorm(x):
    m = jnp.mean(x, axis=-1, keepdims=True)
    d = x - m
    v = jnp.mean(d * d, axis=-1, keepdims=True)
    return d / jnp.sqrt(v + _EPS)


def _dot(a, b):
    return jnp.dot(a, b, preferred_element_type=jnp.float32)


def _dot_nt(a, b):
    return jax.lax.dot_general(a, b, (((1,), (1,)), ((), ())),
                               preferred_element_type=jnp.float32)


@jax.jit
def pallas_adaLN_cond__sliding_block_cached__mixer_channel_mlp__decode_kernel(
    A_x: jax.Array,
    A_k_cache: jax.Array,
    A_v_cache: jax.Array,
    A_wq: jax.Array,
    A_wo: jax.Array,
    B_x: jax.Array,
    B_w1: jax.Array,
    B_b1: jax.Array,
    B_w2: jax.Array,
    B_b2: jax.Array,
    c: jax.Array,
    w_mod: jax.Array,
):
    del B_x
    B, Sq, D = A_x.shape
    _, H, Sk, Dh = A_k_cache.shape
    F = B_w1.shape[1]
    W = min(4096, max(256, Sk // 4))
    HD = H * Dh
    assert (Sq, W, Dh) == (1, 1024, 192) and A_wq.shape == (D, HD) and H % _HG == 0
    assert sum(_W2_CHUNKS) == F and HD % _WO_CHUNKS == 0
    rows = _HG * Dh
    nh = H // _HG
    nblk = B * nh
    bm = rows // _MAJ
    nu = bm // 2
    scale = Dh ** -0.5
    f32, bf16 = jnp.float32, jnp.bfloat16
    w2_off = [sum(_W2_CHUNKS[:i]) for i in range(len(_W2_CHUNKS))]
    wo_rows = HD // _WO_CHUNKS
    n_sems = 4 + 7 + _WO_CHUNKS + len(_W2_CHUNKS)

    def kernel(x_hbm, k_hbm, v_hbm, wq_hbm, wo_hbm, w1_hbm, b1_hbm, w2_hbm, b2_hbm,
               c_hbm, wm_hbm, out_ref,
               x_v, c_v, b1_v, b2_v, wm_v, wq_v, wo_v, w1_v, w2_v,
               kbuf, vbuf, qbd_s, s_s, p_s, o_s, sem):
        def kv_start(a, blk, r, j):
            src, buf = ((k_hbm, kbuf), (v_hbm, vbuf))[a]
            slot = blk % 2
            r8 = r * 8 if isinstance(r, int) else pl.multiple_of(r * 8, 8)
            pltpu.make_async_copy(
                src.at[pl.ds(blk * bm + 2 * j, 2), pl.ds(r8, 8), pl.ds(Sk - W, W)],
                buf.at[slot, pl.ds(2 * j, 2), pl.ds(r8, 8), :],
                sem.at[2 * a + slot]).start(priority=a)

        def kv_wait(a, blk):
            buf = (kbuf, vbuf)[a].at[blk % 2]
            pltpu.make_async_copy(buf, buf, sem.at[2 * a + blk % 2]).wait()

        def pump(m, i, j):
            kb = m + (i + 1) // 8

            @pl.when(kb < nblk)
            def _():
                kv_start(0, kb, (i + 1) % 8, j)

            kv_start(1, m, i, j)

        free_sems = iter(range(4, n_sems))

        def copy(src, dst):
            return pltpu.make_async_copy(src, dst, sem.at[next(free_sems)])

        def row_copy(src, dst, o, n):
            return copy(src.at[pl.ds(o, n), :], dst.at[pl.ds(o, n), :])

        c_cp = copy(c_hbm, c_v)
        x_cp = copy(x_hbm, x_v)
        b1_cp = copy(b1_hbm, b1_v)
        b2_cp = copy(b2_hbm, b2_v)
        wm_cp = copy(wm_hbm, wm_v)
        wq_cp = copy(wq_hbm, wq_v)
        w1_cp = copy(w1_hbm, w1_v)
        wo_cp = [row_copy(wo_hbm, wo_v, j * wo_rows, wo_rows) for j in range(_WO_CHUNKS)]
        w2_cp = [row_copy(w2_hbm, w2_v, o, n) for o, n in zip(w2_off, _W2_CHUNKS)]

        for cp in (wm_cp, c_cp, x_cp, wq_cp, b1_cp, b2_cp, w1_cp):
            cp.start(priority=1)
        for j in range(nu):
            kv_start(0, 0, 0, j)

        wm_cp.wait()
        c_cp.wait()
        x_cp.wait()
        x = x_v[...].astype(f32)
        mod = _dot(jax.nn.silu(c_v[...].astype(f32)).astype(bf16), wm_v[...])
        sa, ca, ga, sb, cb, gb = (mod[:, t * D:(t + 1) * D] for t in range(6))
        h = (_layernorm(x) * (1.0 + ca) + sa).astype(bf16)
        wq_cp.wait()
        row_id = jax.lax.broadcasted_iota(jnp.int32, (_HG, rows), 0)
        col_id = jax.lax.broadcasted_iota(jnp.int32, (_HG, rows), 1)
        diag = jnp.logical_and(col_id >= row_id * Dh, col_id < (row_id + 1) * Dh)
        for hf in range(nh):
            q = _dot(h, wq_v[:, hf * rows:(hf + 1) * rows])
            for b in range(B):
                qbd_s[b * nh + hf] = jnp.where(
                    diag, jnp.broadcast_to(q[b:b + 1, :], (_HG, rows)), 0.0).astype(bf16)

        row2 = jax.lax.broadcasted_iota(jnp.int32, (_HG, 256), 0)
        col2 = jax.lax.broadcasted_iota(jnp.int32, (_HG, 256), 1)

        def attend(n, between):
            slot = n % 2

            def scores(i, carry):
                c0 = pl.multiple_of(i * 256, 256)
                acc = jnp.zeros((_HG, 256), f32)
                for j in range(nu):
                    between(i, j)
                    kt = kbuf[slot, pl.ds(2 * j, 2), :, pl.ds(c0, 256)].reshape(128, 256)
                    acc = acc + _dot(qbd_s[n, :, pl.ds(j * 128, 128)], kt)
                s_s[i] = acc
                return carry

            def values(i, carry):
                for rp in range(3):
                    acc = jnp.zeros((_HG, 256), f32)
                    for t in range(8):
                        between(4 + i, rp * 8 + t)
                        vt = vbuf[slot, pl.ds(12 * i + 4 * rp, 4), :, pl.ds(t * 128, 128)]
                        acc = acc + _dot_nt(p_s[:, pl.ds(t * 128, 128)], vt.reshape(256, 128))
                    lo = (row2 - 4 * i) * Dh - 256 * rp
                    keep = jnp.logical_and(col2 >= lo, col2 < lo + Dh)
                    o_s[(n % nh) * 12 + 3 * i + rp, pl.ds(n // nh, 1), :] = jnp.sum(
                        jnp.where(keep, acc, 0.0), axis=0, keepdims=True)
                return carry

            kv_wait(0, n)
            jax.lax.fori_loop(0, 4, scores, 0)
            s = jnp.concatenate([s_s[t] for t in range(4)], axis=1) * scale
            p = jnp.exp(s - jnp.max(s, axis=-1, keepdims=True))
            p_s[...] = (p / jnp.sum(p, axis=-1, keepdims=True)).astype(bf16)
            kv_wait(1, n)
            jax.lax.fori_loop(0, 4, values, 0)

        def first_period(i, carry):
            for j in range(nu):
                pump(0, i, j)
            return carry

        def period(m, carry):
            attend(m - 1, lambda i, j: pump(m, i, j))
            return carry

        jax.lax.fori_loop(0, 8, first_period, 0)
        jax.lax.fori_loop(1, nblk, period, 0)
        for cp in (*wo_cp, *w2_cp):
            cp.start(priority=1)
        attend(nblk - 1, lambda i, j: None)

        o_all = jnp.concatenate([o_s[t] for t in range(HD // 256)], axis=1).astype(bf16)
        attn = jnp.zeros((B, D), f32)
        for j in range(_WO_CHUNKS):
            wo_cp[j].wait()
            lo, hi = j * wo_rows, (j + 1) * wo_rows
            attn = attn + _dot(o_all[:, lo:hi], wo_v[lo:hi, :])
        x1 = x + ga * attn
        h2 = _layernorm(x1) * (1.0 + cb) + sb
        y = _layernorm(h2).astype(bf16)
        b1_cp.wait()
        b2_cp.wait()
        w1_cp.wait()
        u = _dot(y, w1_v[...]) + b1_v[...].astype(f32).reshape(1, F)
        u = jax.nn.gelu(u, approximate=True).astype(bf16)
        mlp = b2_v[...].astype(f32).reshape(1, D)
        for cp, o, n in zip(w2_cp, w2_off, _W2_CHUNKS):
            cp.wait()
            mlp = mlp + _dot(u[:, o:o + n], w2_v[o:o + n, :])
        out_ref[...] = (x1 + gb * mlp).astype(out_ref.dtype)

    kt = jnp.swapaxes(A_k_cache, 2, 3).reshape(B * HD // _MAJ, _MAJ, Sk)
    vt = jnp.swapaxes(A_v_cache, 2, 3).reshape(B * HD // _MAJ, _MAJ, Sk)

    out = pl.pallas_call(
        kernel,
        out_shape=jax.ShapeDtypeStruct((B, D), A_x.dtype),
        in_specs=[pl.BlockSpec(memory_space=pl.ANY)] * 11,
        out_specs=pl.BlockSpec(memory_space=pltpu.VMEM),
        scratch_shapes=[
            pltpu.VMEM((B, D), bf16),
            pltpu.VMEM((B, D), bf16),
            pltpu.VMEM((F,), bf16),
            pltpu.VMEM((D,), bf16),
            pltpu.VMEM((D, 6 * D), bf16),
            pltpu.VMEM((D, HD), bf16),
            pltpu.VMEM((HD, D), bf16),
            pltpu.VMEM((D, F), bf16),
            pltpu.VMEM((F, D), bf16),
            pltpu.VMEM((2, bm, _MAJ, W), bf16),
            pltpu.VMEM((2, bm, _MAJ, W), bf16),
            pltpu.VMEM((nblk, _HG, rows), bf16),
            pltpu.VMEM((W // 256, _HG, 256), f32),
            pltpu.VMEM((_HG, W), bf16),
            pltpu.VMEM((HD // 256, B, 256), f32),
            pltpu.SemaphoreType.DMA((n_sems,)),
        ],
        compiler_params=pltpu.CompilerParams(
            vmem_limit_bytes=96 * 1024 * 1024,
            disable_bounds_checks=True,
            disable_semaphore_checks=True,
        ),
    )(A_x.reshape(B, D), kt, vt, A_wq, A_wo, B_w1, B_b1, B_w2, B_b2, c, w_mod)
    return out.reshape(B, Sq, D)
```

```python
import functools

import jax
import jax.numpy as jnp
import jax.experimental.pallas as pl
import jax.experimental.pallas.tpu as pltpu

_EPS = 1e-05
_HG = 16
_MAJ = 64
_HM = 80
_OM = 384
_LAG = 26
_W2_CHUNKS = (1024, 384, 128)


def _layernorm(x):
    m = jnp.mean(x, axis=-1, keepdims=True)
    d = x - m
    v = jnp.mean(d * d, axis=-1, keepdims=True)
    return d / jnp.sqrt(v + _EPS)


def _dot(a, b):
    return jnp.dot(a, b, preferred_element_type=jnp.float32)


def _dot_nt(a, b):
    return jax.lax.dot_general(a, b, (((1,), (1,)), ((), ())),
                               preferred_element_type=jnp.float32)


@jax.jit
def pallas_adaLN_cond__sliding_block_cached__mixer_channel_mlp__decode_kernel(
    A_x: jax.Array,
    A_k_cache: jax.Array,
    A_v_cache: jax.Array,
    A_wq: jax.Array,
    A_wo: jax.Array,
    B_x: jax.Array,
    B_w1: jax.Array,
    B_b1: jax.Array,
    B_w2: jax.Array,
    B_b2: jax.Array,
    c: jax.Array,
    w_mod: jax.Array,
):
    del B_x
    B, Sq, D = A_x.shape
    _, H, Sk, Dh = A_k_cache.shape
    F = B_w1.shape[1]
    W = min(4096, max(256, Sk // 4))
    HD = H * Dh
    assert (B, Sq, D, H, Dh, W) == (8, 1, 640, 32, 192, 1024)
    assert A_wq.shape == (D, HD) and sum(_W2_CHUNKS) == F
    rows = _HG * Dh
    nh = H // _HG
    nblk = B * nh
    bm = rows // _MAJ
    ns = bm // 2
    nbody = 8 * nblk
    scale = Dh ** -0.5
    f32, bf16 = jnp.float32, jnp.bfloat16
    w2_off = [sum(_W2_CHUNKS[:i]) for i in range(len(_W2_CHUNKS))]
    q_slot = 4
    sem_wm, sem_wq, sem_wo, sem_free = 4, 5, 6, 9
    n_sems = sem_free + 5 + len(_W2_CHUNKS)

    def kernel(x_hbm, k_hbm, v_hbm, wq_hbm, wo_hbm, w1_hbm, b1_hbm, w2_hbm, b2_hbm,
               c_hbm, wm_hbm, out_ref,
               x_v, c_v, b1_v, b2_v, wqm_v, wo_v, w1_v, w2_v,
               kvbuf, mod_s, h_s, s_s, p_s, o_s, sem):
        def kv_unit(src, gb, t, q):
            blk, slot = gb // 8, 2 * ((gb // 4) % 2) + (gb // 8) % 2
            r8 = (2 * (gb % 4) + t // 12) * 8
            if not isinstance(gb, int):
                r8 = pl.multiple_of(r8, 8)
            j = 2 * (t % 12) + q
            pltpu.make_async_copy(
                src.at[pl.ds(blk * bm + 2 * j, 2), pl.ds(r8, 8), pl.ds(Sk - W, W)],
                kvbuf.at[slot, pl.ds(2 * j, 2), pl.ds(r8, 8), :],
                sem.at[slot]).start(priority=q)

        def wo_unit(gb, t, q):
            r = 12 * (gb - nbody) + (2 * t + q) // 4
            sl = (pl.ds(4 * ((2 * t + q) % 4), 4), pl.ds(pl.multiple_of(r * 8, 8), 8),
                  slice(None))
            pltpu.make_async_copy(wo_hbm.at[sl], wo_v.at[sl],
                                  sem.at[sem_wo + r // 16]).start(priority=q)

        def unit(gb, t, q, last=False):
            if isinstance(gb, int):
                kv_unit((k_hbm, v_hbm)[(gb // 4) % 2], gb, t, q)
            elif not last:
                pl.when((gb // 4) % 2 == 0)(lambda: kv_unit(k_hbm, gb, t, q))
                pl.when((gb // 4) % 2 == 1)(lambda: kv_unit(v_hbm, gb, t, q))
            else:
                pl.when(gb < nbody)(lambda: kv_unit(v_hbm, gb, t, q))
                pl.when(jnp.logical_and(gb >= nbody, gb < nbody + 4))(
                    lambda: wo_unit(gb, t, q))

        def pump(gb, t, last=False):
            unit(gb, t, 0, last)
            unit(gb + (t + _LAG) // ns, (t + _LAG) % ns, 1, last)

        def wait_all(ref, s):
            pltpu.make_async_copy(ref, ref, sem.at[s]).wait()

        free_sems = iter(range(sem_free, n_sems))

        def copy(src, dst):
            return pltpu.make_async_copy(src, dst, sem.at[next(free_sems)])

        c_cp = copy(c_hbm, c_v)
        x_cp = copy(x_hbm, x_v)
        b1_cp = copy(b1_hbm, b1_v)
        b2_cp = copy(b2_hbm, b2_v)
        w1_cp = copy(w1_hbm, w1_v)
        w2_cp = [copy(w2_hbm.at[pl.ds(o, n), :], w2_v.at[pl.ds(o, n), :])
                 for o, n in zip(w2_off, _W2_CHUNKS)]

        def head_unit(src, col0, s, m, nm, r, c0, w, q):
            pltpu.make_async_copy(
                src.at[pl.ds(m, nm), pl.ds(r, 8), pl.ds(c0, w)],
                wqm_v.at[pl.ds(m, nm), pl.ds(r, 8), pl.ds(col0 + c0, w)],
                sem.at[s]).start(priority=q)

        units = [functools.partial(head_unit, wm_hbm, HD, sem_wm, m, 1, r, c0, 3 * D)
                 for r in range(0, _HM, 8) for c0 in (0, 3 * D) for m in range(D // _HM)]
        mod_step = len(units) // 2 + 12
        units += [functools.partial(head_unit, wq_hbm, 0, sem_wq, m, 2, r, c0, 1024)
                  for r in range(0, _HM, 8) for c0 in range(0, HD, 1024)
                  for m in range(0, D // _HM, 2)]
        hi_units = units[0::2]
        lo_units = units[1::2] + [functools.partial(unit, t // ns, t % ns)
                                  for t in range(_LAG)]

        for start in lo_units[:4]:
            start(1)
        for cp in (c_cp, x_cp, b1_cp, b2_cp):
            cp.start(priority=0)
        for start in lo_units[4:_LAG]:
            start(1)
        for t in range(len(hi_units)):
            hi_units[t](0)
            lo_units[t + _LAG](1)
            if t == 8:
                c_cp.wait()
                x_cp.wait()
                x = x_v[...].astype(f32)
                ln_x = _layernorm(x)
                sc = jax.nn.silu(c_v[...].astype(f32)).astype(bf16)
            if t == mod_step:
                wait_all(wqm_v.at[:, :, pl.ds(HD, 6 * D)], sem_wm)
            ct, odd = divmod(t - mod_step, 2)
            if 0 <= ct < 6 * D // 128 and not odd:
                w = wqm_v[:, :, pl.ds(HD + ct * 128, 128)].reshape(D, 128)
                mod_s[:, pl.ds(ct * 128, 128)] = _dot(sc, w)
                if ct == 2 * D // 128 + 1:
                    h_s[...] = (ln_x * (1.0 + mod_s[:, D:2 * D]) + mod_s[:, 0:D]).astype(bf16)

        for t in range(ns):
            pump(0, t)
        wait_all(wqm_v.at[:, :, pl.ds(0, HD)], sem_wq)

        row1 = jax.lax.broadcasted_iota(jnp.int32, (_HG, 128), 0)
        col1 = jax.lax.broadcasted_iota(jnp.int32, (_HG, 128), 1)

        def queries(i, carry):
            h = h_s[...]
            for t in range(12):
                pump(1 + i, 2 * t)
                c0 = pl.multiple_of((12 * i + t) * 128, 128)
                q = _dot(h, wqm_v[:, :, pl.ds(c0, 128)].reshape(D, 128))
                lo = (row1 - 8 * (i % 2)) * Dh - 128 * t
                keep = jnp.logical_and(col1 >= lo, col1 < lo + Dh)
                kt = 12 * (i % 2) + t
                for b in range(B):
                    if b == B // 2:
                        pump(1 + i, 2 * t + 1)
                    tile = jnp.where(keep, jnp.broadcast_to(q[b:b + 1, :], (_HG, 128)), 0.0)
                    kvbuf[q_slot, 3 * (b * nh + i // 2) + kt // 8, pl.ds(0, _HG),
                          pl.ds(pl.multiple_of((kt % 8) * 128, 128), 128)] = tile.astype(bf16)
            return carry

        jax.lax.fori_loop(0, 4, queries, 0)

        row2 = jax.lax.broadcasted_iota(jnp.int32, (_HG, 256), 0)
        col2 = jax.lax.broadcasted_iota(jnp.int32, (_HG, 256), 1)

        def attend(n, last):
            k_slot, v_slot = n % 2, 2 + n % 2

            def scores(i, carry):
                c0 = pl.multiple_of(i * 256, 256)
                acc = jnp.zeros((_HG, 256), f32)
                for t in range(ns):
                    pump(8 * n + 5 + i, t, last)
                    kt = kvbuf[k_slot, pl.ds(2 * t, 2), :, pl.ds(c0, 256)].reshape(128, 256)
                    qt = kvbuf[q_slot, 3 * n + t // 8, pl.ds(0, _HG), pl.ds((t % 8) * 128, 128)]
                    acc = acc + _dot(qt, kt)
                s_s[i] = acc
                return carry

            def values(i, carry):
                for rp in range(3):
                    acc = jnp.zeros((_HG, 256), f32)
                    for t in range(8):
                        pump(8 * n + 9 + i, rp * 8 + t, last)
                        vt = kvbuf[v_slot, pl.ds(12 * i + 4 * rp, 4), :, pl.ds(t * 128, 128)]
                        acc = acc + _dot_nt(p_s[:, pl.ds(t * 128, 128)], vt.reshape(256, 128))
                    lo = (row2 - 4 * i) * Dh - 256 * rp
                    keep = jnp.logical_and(col2 >= lo, col2 < lo + Dh)
                    o_s[(n % nh) * 12 + 3 * i + rp, pl.ds(n // nh, 1), :] = jnp.sum(
                        jnp.where(keep, acc, 0.0), axis=0, keepdims=True)
                if last:
                    @pl.when(i == 1)
                    def _():
                        for cp in (w1_cp, *w2_cp):
                            cp.start(priority=1)
                return carry

            wait_all(kvbuf.at[k_slot], k_slot)
            jax.lax.fori_loop(0, 4, scores, 0)
            s = jnp.concatenate([s_s[t] for t in range(4)], axis=1) * scale
            p = jnp.exp(s - jnp.max(s, axis=-1, keepdims=True))
            p_s[...] = (p / jnp.sum(p, axis=-1, keepdims=True)).astype(bf16)
            wait_all(kvbuf.at[v_slot], v_slot)
            jax.lax.fori_loop(0, 4, values, 0)

        def period(n, carry):
            attend(n, False)
            return carry

        jax.lax.fori_loop(0, nblk - 1, period, 0)
        attend(jnp.int32(nblk - 1), True)

        o_all = jnp.concatenate([o_s[t] for t in range(HD // 256)], axis=1).astype(bf16)
        attn = jnp.zeros((B, D), f32)
        for c3 in range(_OM // 128):
            wait_all(wo_v.at[:, pl.ds(c3 * 128, 128), :], sem_wo + c3)
            oc = jnp.concatenate([o_all[:, m + c3 * 128:m + (c3 + 1) * 128]
                                  for m in range(0, HD, _OM)], axis=1)
            attn = attn + _dot(oc, wo_v[:, pl.ds(c3 * 128, 128), :].reshape(HD // 3, D))
        ga, sb, cb, gb = (mod_s[:, t * D:(t + 1) * D] for t in range(2, 6))
        x1 = x + ga * attn
        h2 = _layernorm(x1) * (1.0 + cb) + sb
        y = _layernorm(h2).astype(bf16)
        b1_cp.wait()
        b2_cp.wait()
        w1_cp.wait()
        u = _dot(y, w1_v[...]) + b1_v[...].astype(f32).reshape(1, F)
        u = jax.nn.gelu(u, approximate=True).astype(bf16)
        mlp = b2_v[...].astype(f32).reshape(1, D)
        for cp, o, n in zip(w2_cp, w2_off, _W2_CHUNKS):
            cp.wait()
            mlp = mlp + _dot(u[:, o:o + n], w2_v[o:o + n, :])
        out_ref[...] = (x1 + gb * mlp).astype(out_ref.dtype)

    kt = jnp.swapaxes(A_k_cache, 2, 3).reshape(B * HD // _MAJ, _MAJ, Sk)
    vt = jnp.swapaxes(A_v_cache, 2, 3).reshape(B * HD // _MAJ, _MAJ, Sk)

    out = pl.pallas_call(
        kernel,
        out_shape=jax.ShapeDtypeStruct((B, D), A_x.dtype),
        in_specs=[pl.BlockSpec(memory_space=pl.ANY)] * 11,
        out_specs=pl.BlockSpec(memory_space=pltpu.VMEM),
        scratch_shapes=[
            pltpu.VMEM((B, D), bf16),
            pltpu.VMEM((B, D), bf16),
            pltpu.VMEM((F,), bf16),
            pltpu.VMEM((D,), bf16),
            pltpu.VMEM((D // _HM, _HM, HD + 6 * D), bf16),
            pltpu.VMEM((HD // _OM, _OM, D), bf16),
            pltpu.VMEM((D, F), bf16),
            pltpu.VMEM((F, D), bf16),
            pltpu.VMEM((5, bm, _MAJ, W), bf16),
            pltpu.VMEM((B, 6 * D), f32),
            pltpu.VMEM((B, D), bf16),
            pltpu.VMEM((W // 256, _HG, 256), f32),
            pltpu.VMEM((_HG, W), bf16),
            pltpu.VMEM((HD // 256, B, 256), f32),
            pltpu.SemaphoreType.DMA((n_sems,)),
        ],
        compiler_params=pltpu.CompilerParams(
            vmem_limit_bytes=96 * 1024 * 1024,
            disable_bounds_checks=True,
            disable_semaphore_checks=True,
        ),
    )(A_x.reshape(B, D), kt, vt, A_wq.reshape(D // _HM, _HM, HD),
      A_wo.reshape(HD // _OM, _OM, D), B_w1, B_b1, B_w2, B_b2, c,
      w_mod.reshape(D // _HM, _HM, 6 * D))
    return out.reshape(B, Sq, D)
```

```python
import functools

import jax
import jax.numpy as jnp
import jax.experimental.pallas as pl
import jax.experimental.pallas.tpu as pltpu

_EPS = 1e-05
_HG = 16
_MAJ = 64
_HM = 80
_OM = 384
_W1M = 160
_LAG = 26
_NVP = 10


def _layernorm(x):
    m = jnp.mean(x, axis=-1, keepdims=True)
    d = x - m
    v = jnp.mean(d * d, axis=-1, keepdims=True)
    return d / jnp.sqrt(v + _EPS)


def _dot(a, b):
    return jnp.dot(a, b, preferred_element_type=jnp.float32)


def _dot_nt(a, b):
    return jax.lax.dot_general(a, b, (((1,), (1,)), ((), ())),
                               preferred_element_type=jnp.float32)


@jax.jit
def pallas_adaLN_cond__sliding_block_cached__mixer_channel_mlp__decode_kernel(
    A_x: jax.Array,
    A_k_cache: jax.Array,
    A_v_cache: jax.Array,
    A_wq: jax.Array,
    A_wo: jax.Array,
    B_x: jax.Array,
    B_w1: jax.Array,
    B_b1: jax.Array,
    B_w2: jax.Array,
    B_b2: jax.Array,
    c: jax.Array,
    w_mod: jax.Array,
):
    del B_x
    B, Sq, D = A_x.shape
    _, H, Sk, Dh = A_k_cache.shape
    F = B_w1.shape[1]
    W = min(4096, max(256, Sk // 4))
    HD = H * Dh
    assert (B, Sq, D, H, Dh, W, F) == (8, 1, 640, 32, 192, 1024, 1536)
    assert A_wq.shape == (D, HD)
    nh = H // _HG
    nblk = B * nh
    bm = _HG * Dh // _MAJ
    ns = bm // 2
    nbody = 8 * nblk
    n_wo, n_w2 = HD // _OM, F // _OM
    scale = Dh ** -0.5
    f32, bf16 = jnp.float32, jnp.bfloat16
    a_q = 4 * bm
    a_wo = a_q + bm
    a_w2 = a_wo + HD // _MAJ
    a_end = a_w2 + F // _MAJ
    sem_wm, sem_wq, sem_wo, sem_w1, sem_w2, sem_small = 4, 5, 6, 9, 10, 14
    partial = functools.partial

    def kernel(x_hbm, k_hbm, v_hbm, wq_hbm, wo_hbm, w1_hbm, b1_hbm, w2_hbm, b2_hbm,
               c_hbm, wm_hbm, out_ref,
               x_v, c_v, b1_v, b2_v, wqm_v, w1_v, arena, mod_s, h_s, s_s, p_s, o_s, sem):
        def aligned(v, n):
            return v if isinstance(v, int) else pl.multiple_of(v, n)

        def kv_unit(src, gb, t, q):
            blk = gb >> 3
            slot = ((gb >> 1) & 2) + (blk & 1)
            r8 = aligned((2 * (gb & 3) + t // 12) * 8, 8)
            j = 2 * (t % 12) + q
            pltpu.make_async_copy(
                src.at[pl.ds(blk * bm + 2 * j, 2), pl.ds(r8, 8), pl.ds(Sk - W, W)],
                arena.at[pl.ds(slot * bm + 2 * j, 2), pl.ds(r8, 8), :],
                sem.at[slot]).start(priority=q)

        def quad_unit(src, base, nmaj, s0, r, quad, q):
            pltpu.make_async_copy(
                src.at[pl.ds(4 * quad, 4), pl.ds(aligned(r * 8, 8), 8), :],
                arena.at[pl.ds(base + (r >> 3) * nmaj + 4 * quad, 4),
                         pl.ds(aligned((r & 7) * 8, 8), 8), pl.ds(0, D)],
                sem.at[s0 + (r >> 4)]).start(priority=q)

        def wo_unit(s_even, s, q):
            u = 2 * s + q
            quad_unit(wo_hbm, a_wo, n_wo, sem_wo, (s_even >> 1) + u // 4, u % 4, q)

        def strip_unit(src, dst, col0, s, m, r, c0, w, q):
            pltpu.make_async_copy(src.at[m, pl.ds(r, 8), pl.ds(c0, w)],
                                  dst.at[m, pl.ds(r, 8), pl.ds(col0 + c0, w)],
                                  sem.at[s]).start(priority=q)

        def unit(gb, t, q, last=False):
            if isinstance(gb, int):
                kv_unit((k_hbm, v_hbm)[(gb >> 2) & 1], gb, t, q)
            elif not last:
                pl.when((gb & 4) == 0)(lambda: kv_unit(k_hbm, gb, t, q))
                pl.when((gb & 4) != 0)(lambda: kv_unit(v_hbm, gb, t, q))
            else:
                pl.when(gb < nbody)(lambda: kv_unit(v_hbm, gb, t, q))
                pl.when(gb >= nbody)(lambda: wo_unit(ns * (gb - nbody), t, q))

        def pump(gb, t, last=False):
            unit(gb, t, 0, last)
            unit(gb + (t + _LAG) // ns, (t + _LAG) % ns, 1, last)

        def wait_all(ref, s):
            pltpu.make_async_copy(ref, ref, sem.at[s]).wait()

        c_cp, x_cp, b1_cp, b2_cp = (
            pltpu.make_async_copy(src, dst, sem.at[sem_small + i]) for i, (src, dst) in
            enumerate(((c_hbm, c_v), (x_hbm, x_v), (b1_hbm, b1_v), (b2_hbm, b2_v))))

        units = [partial(strip_unit, wm_hbm, wqm_v, HD, sem_wm, m, r, c0, 3 * D)
                 for r in range(0, _HM, 8) for c0 in (0, 3 * D) for m in range(D // _HM)]
        mod_step = len(units) // 2 + 12
        units += [partial(strip_unit, wq_hbm, wqm_v, 0, sem_wq,
                          *divmod(g // 3 * 8, _HM), g % 3 * 2048, 2048)
                  for g0 in range(16) for g in range(g0, D // 8 * 3, 16)]
        hi = units[0::2]
        lo = units[1::2] + [partial(unit, t // ns, t % ns) for t in range(_LAG)]

        for start in lo[:4]:
            start(1)
        for cp in (c_cp, x_cp, b1_cp, b2_cp):
            cp.start(priority=0)
        for start in lo[4:_LAG]:
            start(1)
        for t in range(len(hi)):
            hi[t](0)
            lo[t + _LAG](1)
            if t == 8:
                c_cp.wait()
                x_cp.wait()
                x = x_v[...].astype(f32)
                ln_x = _layernorm(x)
                sc = jax.nn.silu(c_v[...].astype(f32)).astype(bf16)
            if t == mod_step:
                wait_all(wqm_v.at[:, :, pl.ds(HD, 6 * D)], sem_wm)
            ct, odd = divmod(t - mod_step, 2)
            if 0 <= ct < 6 * D // 128 and not odd:
                w = wqm_v[:, :, pl.ds(HD + ct * 128, 128)].reshape(D, 128)
                mod_s[:, pl.ds(ct * 128, 128)] = _dot(sc, w)
                if ct == 2 * D // 128 + 1:
                    h_s[...] = (ln_x * (1.0 + mod_s[:, D:2 * D]) + mod_s[:, 0:D]).astype(bf16)

        for t in range(ns):
            pump(0, t)
        wait_all(wqm_v.at[:, :, pl.ds(0, HD)], sem_wq)

        row1 = jax.lax.broadcasted_iota(jnp.int32, (_HG, 128), 0)
        col1 = jax.lax.broadcasted_iota(jnp.int32, (_HG, 128), 1)

        def queries(i, carry):
            h = h_s[...]
            for t in range(12):
                pump(1 + i, 2 * t)
                c0 = pl.multiple_of((12 * i + t) * 128, 128)
                q = _dot(h, wqm_v[:, :, pl.ds(c0, 128)].reshape(D, 128))
                first = (row1 - 8 * (i & 1)) * Dh - 128 * t
                keep = jnp.logical_and(col1 >= first, col1 < first + Dh)
                kt = 12 * (i & 1) + t
                for b in range(B):
                    if b == B // 2:
                        pump(1 + i, 2 * t + 1)
                    tile = jnp.where(keep, jnp.broadcast_to(q[b:b + 1, :], (_HG, 128)), 0.0)
                    arena[a_q + 3 * (b * nh + (i >> 1)) + (kt >> 3), pl.ds(0, _HG),
                          pl.ds(pl.multiple_of((kt & 7) * 128, 128), 128)] = tile.astype(bf16)
            return carry

        jax.lax.fori_loop(0, 4, queries, 0)

        row2 = jax.lax.broadcasted_iota(jnp.int32, (_HG, 256), 0)
        col2 = jax.lax.broadcasted_iota(jnp.int32, (_HG, 256), 1)

        def attend(n, last):
            k_slot, v_slot = n & 1, 2 + (n & 1)

            def scores(i, carry):
                c0 = pl.multiple_of(i * 256, 256)
                acc = jnp.zeros((_HG, 256), f32)
                for t in range(ns):
                    pump(8 * n + 5 + i, t, last)
                    kt = arena[pl.ds(k_slot * bm + 2 * t, 2), :, pl.ds(c0, 256)]
                    qt = arena[a_q + 3 * n + t // 8, pl.ds(0, _HG), pl.ds((t % 8) * 128, 128)]
                    acc = acc + _dot(qt, kt.reshape(128, 256))
                s_s[i] = acc
                return carry

            def values(i, carry):
                for rp in range(3):
                    acc = jnp.zeros((_HG, 256), f32)
                    for t in range(8):
                        z = rp * 8 + t
                        if not last:
                            pump(8 * n + 9 + i, z)
                        elif z * _NVP // ns != (z + 1) * _NVP // ns:
                            wo_unit(_NVP * i, ns + z * _NVP // ns, 0)
                            wo_unit(_NVP * i, ns + z * _NVP // ns + _LAG, 1)
                        vt = arena[pl.ds(v_slot * bm + 12 * i + 4 * rp, 4), :,
                                   pl.ds(t * 128, 128)]
                        acc = acc + _dot_nt(p_s[:, pl.ds(t * 128, 128)], vt.reshape(256, 128))
                    first = (row2 - 4 * i) * Dh - 256 * rp
                    keep = jnp.logical_and(col2 >= first, col2 < first + Dh)
                    o_s[(n & 1) * 12 + 3 * i + rp, pl.ds(n >> 1, 1), :] = jnp.sum(
                        jnp.where(keep, acc, 0.0), axis=0, keepdims=True)
                return carry

            wait_all(arena.at[pl.ds(k_slot * bm, bm)], k_slot)
            jax.lax.fori_loop(0, 4, scores, 0)
            s = jnp.concatenate([s_s[t] for t in range(4)], axis=1) * scale
            p = jnp.exp(s - jnp.max(s, axis=-1, keepdims=True))
            p_s[...] = (p / jnp.sum(p, axis=-1, keepdims=True)).astype(bf16)
            wait_all(arena.at[pl.ds(v_slot * bm, bm)], v_slot)
            jax.lax.fori_loop(0, 4, values, 0)

        def period(n, carry):
            attend(n, False)
            return carry

        jax.lax.fori_loop(0, nblk - 1, period, 0)
        attend(nblk - 1, True)

        def w2_block(m, rb, s, q):
            pltpu.make_async_copy(w2_hbm.at[m, pl.ds(rb * _MAJ, _MAJ), :],
                                  arena.at[a_w2 + rb * n_w2 + m, :, pl.ds(0, D)],
                                  sem.at[s]).start(priority=q)

        units = [partial(quad_unit, wo_hbm, a_wo, n_wo, sem_wo, u // 4, u % 4)
                 for u in range(HD // 32)]
        w1_units = [partial(strip_unit, w1_hbm, w1_v, 0, sem_w1, m, r, 0, F)
                    for r in range(0, _W1M, 8) for m in range(D // _W1M)]
        w2_units = [partial(quad_unit, w2_hbm, a_w2, n_w2, sem_w2, r, 0) for r in range(32)]
        for r in range(16):
            units += w1_units[5 * r:5 * r + 5] + [w2_units[r]]
        hi = units[0::2]
        lo = (units[1::2] + w2_units[16:]
              + [partial(w2_block, m, rb, sem_w2 + 2) for m in range(3) for rb in (4, 5)]
              + [partial(w2_block, 3, rb, sem_w2 + 3) for rb in (4, 5)])

        def ktile(base, nmaj, m, c3):
            return jnp.concatenate(
                [arena[base + (2 * c3 + e) * nmaj + m, :, pl.ds(0, D)] for e in range(2)],
                axis=0)

        s0 = ns + 4 * _NVP
        chunk_step = (s0, s0 + n_wo, HD // 64 + 8)
        attn = jnp.zeros((B, D), f32)
        for t in range(s0, len(hi)):
            if t in chunk_step:
                c3 = chunk_step.index(t)
                wait_all(arena.at[pl.ds(a_wo + 2 * n_wo * c3, 2 * n_wo), :, pl.ds(0, D)],
                         sem_wo + c3)
            hi[t](0)
            if t + _LAG < len(lo):
                lo[t + _LAG](1)
            m = t - chunk_step[c3]
            if m < n_wo:
                col = m * _OM + c3 * 128
                o_t = o_s[col // 256, :, pl.ds(col % 256, 128)].astype(bf16)
                attn = attn + _dot(o_t, ktile(a_wo, n_wo, m, c3))
            if (c3, m) == (2, n_wo - 1):
                ga, sb, cb, gb = (mod_s[:, k * D:(k + 1) * D] for k in range(2, 6))
                x1 = x + ga * attn
                h2 = _layernorm(x1) * (1.0 + cb) + sb
                y = _layernorm(h2).astype(bf16)
        assert len(lo) <= len(hi) + _LAG

        b1_cp.wait()
        b2_cp.wait()
        wait_all(w1_v, sem_w1)
        u = _dot(y, w1_v[...].reshape(D, F)) + b1_v[...].astype(f32).reshape(1, F)
        u = jax.nn.gelu(u, approximate=True).astype(bf16)

        def w2_dot(tiles):
            lhs = [u[:, m * _OM + c3 * 128:m * _OM + (c3 + 1) * 128] for m, c3 in tiles]
            rhs = [ktile(a_w2, n_w2, m, c3) for m, c3 in tiles]
            return _dot(jnp.concatenate(lhs, axis=1), jnp.concatenate(rhs, axis=0))

        for c3 in range(2):
            wait_all(arena.at[pl.ds(a_w2 + 2 * n_w2 * c3, 2 * n_w2), :, pl.ds(0, D)],
                     sem_w2 + c3)
        mlp = b2_v[...].astype(f32).reshape(1, D)
        mlp = mlp + w2_dot([(m, c3) for c3 in range(2) for m in range(n_w2)])
        for rb in (4, 5):
            wait_all(arena.at[pl.ds(a_w2 + rb * n_w2, 3), :, pl.ds(0, D)], sem_w2 + 2)
        mlp = mlp + w2_dot([(m, 2) for m in range(3)])
        for rb in (4, 5):
            wait_all(arena.at[a_w2 + rb * n_w2 + 3, :, pl.ds(0, D)], sem_w2 + 3)
        mlp = mlp + w2_dot([(3, 2)])
        out_ref[...] = (x1 + gb * mlp).astype(out_ref.dtype)

    kt = jnp.swapaxes(A_k_cache, 2, 3).reshape(B * HD // _MAJ, _MAJ, Sk)
    vt = jnp.swapaxes(A_v_cache, 2, 3).reshape(B * HD // _MAJ, _MAJ, Sk)

    out = pl.pallas_call(
        kernel,
        out_shape=jax.ShapeDtypeStruct((B, D), A_x.dtype),
        in_specs=[pl.BlockSpec(memory_space=pl.ANY)] * 11,
        out_specs=pl.BlockSpec(memory_space=pltpu.VMEM),
        scratch_shapes=[
            pltpu.VMEM((B, D), bf16),
            pltpu.VMEM((B, D), bf16),
            pltpu.VMEM((F,), bf16),
            pltpu.VMEM((D,), bf16),
            pltpu.VMEM((D // _HM, _HM, HD + 6 * D), bf16),
            pltpu.VMEM((D // _W1M, _W1M, F), bf16),
            pltpu.VMEM((a_end, _MAJ, W), bf16),
            pltpu.VMEM((B, 6 * D), f32),
            pltpu.VMEM((B, D), bf16),
            pltpu.VMEM((W // 256, _HG, 256), f32),
            pltpu.VMEM((_HG, W), bf16),
            pltpu.VMEM((HD // 256, B, 256), f32),
            pltpu.SemaphoreType.DMA((sem_small + 4,)),
        ],
        compiler_params=pltpu.CompilerParams(
            vmem_limit_bytes=96 * 1024 * 1024,
            disable_bounds_checks=True,
            disable_semaphore_checks=True,
        ),
    )(A_x.reshape(B, D), kt, vt, A_wq.reshape(D // _HM, _HM, HD),
      A_wo.reshape(n_wo, _OM, D), B_w1.reshape(D // _W1M, _W1M, F), B_b1,
      B_w2.reshape(n_w2, _OM, D), B_b2, c, w_mod.reshape(D // _HM, _HM, 6 * D))
    return out.reshape(B, Sq, D)
```

```python
import functools

import jax
import jax.numpy as jnp
import jax.experimental.pallas as pl
import jax.experimental.pallas.tpu as pltpu

_EPS = 1e-05
_HG = 16
_MAJ = 64
_HM = 80
_OM = 384
_W1M = 160
_LAG = 25
_NVP = 10
_PAIRS = ([(0, 1), (2, 3)]
          + [(o + a, o + b) for o in range(4, 44, 8)
             for a, b in ((0, 6), (3, 5), (1, 7), (2, 4))]
          + [(44, 45), (46, 47)])


def _place(m0, e):
    hi = ((m0 >> 2) + 1) & 1
    inner = m0 - 4 * hi + 2 * (e ^ (2 * hi)) + hi
    if isinstance(m0, int):
        return m0 + e if m0 in (0, 44) else inner
    return jnp.where(jnp.logical_or(m0 == 0, m0 == 44), m0 + e, inner)


def _layernorm(x):
    m = jnp.mean(x, axis=-1, keepdims=True)
    d = x - m
    v = jnp.mean(d * d, axis=-1, keepdims=True)
    return d / jnp.sqrt(v + _EPS)


def _dot(a, b):
    return jnp.dot(a, b, preferred_element_type=jnp.float32)


def _dot_nt(a, b):
    return jax.lax.dot_general(a, b, (((1,), (1,)), ((), ())),
                               preferred_element_type=jnp.float32)


@jax.jit
def pallas_adaLN_cond__sliding_block_cached__mixer_channel_mlp__decode_kernel(
    A_x: jax.Array,
    A_k_cache: jax.Array,
    A_v_cache: jax.Array,
    A_wq: jax.Array,
    A_wo: jax.Array,
    B_x: jax.Array,
    B_w1: jax.Array,
    B_b1: jax.Array,
    B_w2: jax.Array,
    B_b2: jax.Array,
    c: jax.Array,
    w_mod: jax.Array,
):
    del B_x
    B, Sq, D = A_x.shape
    _, H, Sk, Dh = A_k_cache.shape
    F = B_w1.shape[1]
    W = min(4096, max(256, Sk // 4))
    HD = H * Dh
    assert (B, Sq, D, H, Dh, W, F) == (8, 1, 640, 32, 192, 1024, 1536)
    assert A_wq.shape == (D, HD)
    nh = H // _HG
    nblk = B * nh
    bm = _HG * Dh // _MAJ
    ns = bm // 2
    nbody = 8 * nblk
    n_wo, n_w2 = HD // _OM, F // _OM
    scale = Dh ** -0.5
    f32, bf16 = jnp.float32, jnp.bfloat16
    a_q = 4 * bm
    a_wo = a_q + bm
    a_w2 = a_wo + HD // _MAJ
    a_end = a_w2 + F // _MAJ
    sem_wm, sem_wq, sem_wo, sem_w1, sem_w2, sem_small = 4, 5, 6, 9, 10, 14
    partial = functools.partial

    def kernel(x_hbm, k2_hbm, k6_hbm, v2_hbm, v6_hbm, wq_hbm, wo_hbm, w1_hbm, b1_hbm,
               w2_hbm, b2_hbm, c_hbm, wm_hbm, out_ref,
               x_v, c_v, b1_v, b2_v, wqm_v, w1_v, arena, mod_s, h_s, s_s, p_s, o_s, sem):
        k_hbm, v_hbm = (k2_hbm, k6_hbm), (v2_hbm, v6_hbm)

        def aligned(v, n):
            return v if isinstance(v, int) else pl.multiple_of(v, n)

        def kv_unit(src, gb, t, q):
            blk = gb >> 3
            slot = ((gb >> 1) & 2) + (blk & 1)
            r8 = aligned((2 * (gb & 3) + t // 12) * 8, 8)
            m, m2 = _PAIRS[2 * (t % 12) + q]
            pos = _place(m & ~3, m & 3)
            assert _place(m2 & ~3, m2 & 3) == pos + 1
            by2, by6 = src
            if m2 - m == 1:
                pair = by2.at[blk * (bm // 2) + m // 2]
            elif m2 - m == 2:
                pair = by2.at[pl.ds(blk * (bm // 2) + m // 2, 2), m % 2]
            else:
                pair = by6.at[pl.ds(blk * (bm // 6) + m // 6, 2), m % 6]
            pltpu.make_async_copy(
                pair.at[:, pl.ds(r8, 8), pl.ds(Sk - W, W)],
                arena.at[pl.ds(slot * bm + pos, 2), pl.ds(r8, 8), :],
                sem.at[slot]).start(priority=q)

        def quad_unit(src, base, nmaj, s0, r, quad, q):
            pltpu.make_async_copy(
                src.at[pl.ds(4 * quad, 4), pl.ds(aligned(r * 8, 8), 8), :],
                arena.at[pl.ds(base + (r >> 3) * nmaj + 4 * quad, 4),
                         pl.ds(aligned((r & 7) * 8, 8), 8), pl.ds(0, D)],
                sem.at[s0 + (r >> 4)]).start(priority=q)

        def wo_unit(s_even, s, q):
            u = 2 * s + q
            quad_unit(wo_hbm, a_wo, n_wo, sem_wo, (s_even >> 1) + u // 4, u % 4, q)

        def strip_unit(src, dst, col0, s, m, r, c0, w, q):
            pltpu.make_async_copy(src.at[m, pl.ds(r, 8), pl.ds(c0, w)],
                                  dst.at[m, pl.ds(r, 8), pl.ds(col0 + c0, w)],
                                  sem.at[s]).start(priority=q)

        def unit(gb, t, q, last=False):
            if isinstance(gb, int):
                kv_unit((k_hbm, v_hbm)[(gb >> 2) & 1], gb, t, q)
            elif not last:
                pl.when((gb & 4) == 0)(lambda: kv_unit(k_hbm, gb, t, q))
                pl.when((gb & 4) != 0)(lambda: kv_unit(v_hbm, gb, t, q))
            else:
                pl.when(gb < nbody)(lambda: kv_unit(v_hbm, gb, t, q))
                pl.when(gb >= nbody)(lambda: wo_unit(ns * (gb - nbody), t, q))

        def pump(gb, t, last=False):
            unit(gb, t, 0, last)
            unit(gb + (t + _LAG) // ns, (t + _LAG) % ns, 1, last)

        def wait_all(ref, s):
            pltpu.make_async_copy(ref, ref, sem.at[s]).wait()

        c_cp, x_cp, b1_cp, b2_cp = (
            pltpu.make_async_copy(src, dst, sem.at[sem_small + i]) for i, (src, dst) in
            enumerate(((c_hbm, c_v), (x_hbm, x_v), (b1_hbm, b1_v), (b2_hbm, b2_v))))

        units = [partial(strip_unit, wm_hbm, wqm_v, HD, sem_wm, m, r, c0, 3 * D)
                 for r in range(0, _HM, 8) for c0 in (0, 3 * D) for m in range(D // _HM)]
        mod_step = len(units) // 2 + 12
        units += [partial(strip_unit, wq_hbm, wqm_v, 0, sem_wq,
                          *divmod(g // 3 * 8, _HM), g % 3 * 2048, 2048)
                  for g0 in range(16) for g in range(g0, D // 8 * 3, 16)]
        hi = units[0::2]
        lo = units[1::2] + [partial(unit, t // ns, t % ns) for t in range(_LAG)]

        for start in lo[:4]:
            start(1)
        for cp in (c_cp, x_cp, b1_cp, b2_cp):
            cp.start(priority=0)
        for start in lo[4:_LAG]:
            start(1)
        for t in range(len(hi)):
            hi[t](0)
            lo[t + _LAG](1)
            if t == 8:
                c_cp.wait()
                x_cp.wait()
                x = x_v[...].astype(f32)
                ln_x = _layernorm(x)
                sc = jax.nn.silu(c_v[...].astype(f32)).astype(bf16)
            if t == mod_step:
                wait_all(wqm_v.at[:, :, pl.ds(HD, 6 * D)], sem_wm)
            ct, odd = divmod(t - mod_step, 2)
            if 0 <= ct < 6 * D // 128 and not odd:
                w = wqm_v[:, :, pl.ds(HD + ct * 128, 128)].reshape(D, 128)
                mod_s[:, pl.ds(ct * 128, 128)] = _dot(sc, w)
                if ct == 2 * D // 128 + 1:
                    h_s[...] = (ln_x * (1.0 + mod_s[:, D:2 * D]) + mod_s[:, 0:D]).astype(bf16)

        for t in range(ns):
            pump(0, t)
        wait_all(wqm_v.at[:, :, pl.ds(0, HD)], sem_wq)

        row1 = jax.lax.broadcasted_iota(jnp.int32, (_HG, 128), 0)
        col1 = jax.lax.broadcasted_iota(jnp.int32, (_HG, 128), 1)

        def queries(i, carry):
            h = h_s[...]
            for t in range(12):
                pump(1 + i, 2 * t)
                c0 = pl.multiple_of((12 * i + t) * 128, 128)
                q = _dot(h, wqm_v[:, :, pl.ds(c0, 128)].reshape(D, 128))
                first = (row1 - 8 * (i & 1)) * Dh - 128 * t
                keep = jnp.logical_and(col1 >= first, col1 < first + Dh)
                kt = 12 * (i & 1) + t
                for b in range(B):
                    if b == B // 2:
                        pump(1 + i, 2 * t + 1)
                    tile = jnp.where(keep, jnp.broadcast_to(q[b:b + 1, :], (_HG, 128)), 0.0)
                    arena[a_q + 3 * (b * nh + (i >> 1)) + (kt >> 3), pl.ds(0, _HG),
                          pl.ds(pl.multiple_of((kt & 7) * 128, 128), 128)] = tile.astype(bf16)
            return carry

        jax.lax.fori_loop(0, 4, queries, 0)

        row2 = jax.lax.broadcasted_iota(jnp.int32, (_HG, 256), 0)
        col2 = jax.lax.broadcasted_iota(jnp.int32, (_HG, 256), 1)

        def attend(n, last):
            k_slot, v_slot = n & 1, 2 + (n & 1)

            def scores(i, carry):
                c0 = pl.multiple_of(i * 256, 256)
                acc = jnp.zeros((_HG, 256), f32)
                for t in range(ns):
                    pump(8 * n + 5 + i, t, last)
                    kt = [arena[k_slot * bm + _place(m & ~3, m & 3), :, pl.ds(c0, 256)]
                          for m in (2 * t, 2 * t + 1)]
                    qt = arena[a_q + 3 * n + t // 8, pl.ds(0, _HG), pl.ds((t % 8) * 128, 128)]
                    acc = acc + _dot(qt, jnp.concatenate(kt, axis=0))
                s_s[i] = acc
                return carry

            def values(i, carry):
                for rp in range(3):
                    acc = jnp.zeros((_HG, 256), f32)
                    pos = [v_slot * bm + _place(12 * i + 4 * rp, e) for e in range(4)]
                    for t in range(8):
                        z = rp * 8 + t
                        if not last:
                            pump(8 * n + 9 + i, z)
                        elif z * _NVP // ns != (z + 1) * _NVP // ns:
                            wo_unit(_NVP * i, ns + z * _NVP // ns, 0)
                            wo_unit(_NVP * i, ns + z * _NVP // ns + _LAG, 1)
                        vt = [arena[m, :, pl.ds(t * 128, 128)] for m in pos]
                        acc = acc + _dot_nt(p_s[:, pl.ds(t * 128, 128)],
                                            jnp.concatenate(vt, axis=0))
                    first = (row2 - 4 * i) * Dh - 256 * rp
                    keep = jnp.logical_and(col2 >= first, col2 < first + Dh)
                    o_s[(n & 1) * 12 + 3 * i + rp, pl.ds(n >> 1, 1), :] = jnp.sum(
                        jnp.where(keep, acc, 0.0), axis=0, keepdims=True)
                return carry

            wait_all(arena.at[pl.ds(k_slot * bm, bm)], k_slot)
            jax.lax.fori_loop(0, 4, scores, 0)
            s = jnp.concatenate([s_s[t] for t in range(4)], axis=1) * scale
            p = jnp.exp(s - jnp.max(s, axis=-1, keepdims=True))
            p_s[...] = (p / jnp.sum(p, axis=-1, keepdims=True)).astype(bf16)
            wait_all(arena.at[pl.ds(v_slot * bm, bm)], v_slot)
            jax.lax.fori_loop(0, 4, values, 0)

        def period(n, carry):
            attend(n, False)
            return carry

        jax.lax.fori_loop(0, nblk - 1, period, 0)
        attend(nblk - 1, True)

        def w2_block(m, rb):
            return pltpu.make_async_copy(w2_hbm.at[m, pl.ds(rb * _MAJ, _MAJ), :],
                                         arena.at[a_w2 + rb * n_w2 + m, :, pl.ds(0, D)],
                                         sem.at[sem_w2 + 2 + m // 3])

        w2_blocks = [w2_block(m, rb) for m in range(n_w2) for rb in (4, 5)]
        units = [partial(quad_unit, wo_hbm, a_wo, n_wo, sem_wo, u // 4, u % 4)
                 for u in range(HD // 32)]
        w1_units = [partial(strip_unit, w1_hbm, w1_v, 0, sem_w1, m, r, 0, F)
                    for r in range(0, _W1M, 8) for m in range(D // _W1M)]
        w2_units = [partial(quad_unit, w2_hbm, a_w2, n_w2, sem_w2, r, 0) for r in range(32)]
        for r in range(16):
            units += w1_units[5 * r:5 * r + 5] + [w2_units[r]]
        hi = units[0::2]
        lo = units[1::2] + w2_units[16:] + [cp.start for cp in w2_blocks]

        def ktile(base, nmaj, m, c3):
            return jnp.concatenate(
                [arena[base + (2 * c3 + e) * nmaj + m, :, pl.ds(0, D)] for e in range(2)],
                axis=0)

        s0 = ns + 4 * _NVP
        chunk_step = (s0, s0 + n_wo, HD // 64 + 8)
        attn = jnp.zeros((B, D), f32)
        for t in range(s0, len(hi)):
            if t in chunk_step:
                c3 = chunk_step.index(t)
                wait_all(arena.at[pl.ds(a_wo + 2 * n_wo * c3, 2 * n_wo), :, pl.ds(0, D)],
                         sem_wo + c3)
            hi[t](0)
            if t + _LAG < len(lo):
                lo[t + _LAG](1)
            m = t - chunk_step[c3]
            if m < n_wo:
                col = m * _OM + c3 * 128
                o_t = o_s[col // 256, :, pl.ds(col % 256, 128)].astype(bf16)
                attn = attn + _dot(o_t, ktile(a_wo, n_wo, m, c3))
            if (c3, m) == (2, n_wo - 1):
                ga, sb, cb, gb = (mod_s[:, k * D:(k + 1) * D] for k in range(2, 6))
                x1 = x + ga * attn
                h2 = _layernorm(x1) * (1.0 + cb) + sb
                y = _layernorm(h2).astype(bf16)
        for start in lo[len(hi) + _LAG:]:
            start(1)

        b1_cp.wait()
        b2_cp.wait()
        wait_all(w1_v, sem_w1)
        u = _dot(y, w1_v[...].reshape(D, F)) + b1_v[...].astype(f32).reshape(1, F)
        u = jax.nn.gelu(u, approximate=True).astype(bf16)

        def w2_dot(tiles):
            lhs = [u[:, m * _OM + c3 * 128:m * _OM + (c3 + 1) * 128] for m, c3 in tiles]
            rhs = [ktile(a_w2, n_w2, m, c3) for m, c3 in tiles]
            return _dot(jnp.concatenate(lhs, axis=1), jnp.concatenate(rhs, axis=0))

        for c3 in range(2):
            wait_all(arena.at[pl.ds(a_w2 + 2 * n_w2 * c3, 2 * n_w2), :, pl.ds(0, D)],
                     sem_w2 + c3)
        mlp = b2_v[...].astype(f32).reshape(1, D)
        mlp = mlp + w2_dot([(m, c3) for c3 in range(2) for m in range(n_w2)])
        for cp in w2_blocks[:6]:
            cp.wait()
        mlp = mlp + w2_dot([(m, 2) for m in range(3)])
        for cp in w2_blocks[6:]:
            cp.wait()
        mlp = mlp + w2_dot([(3, 2)])
        out_ref[...] = (x1 + gb * mlp).astype(out_ref.dtype)

    kv_views = [jnp.swapaxes(a, 2, 3).reshape(nblk * bm // g, g, _MAJ, Sk)
                for a in (A_k_cache, A_v_cache) for g in (2, 6)]

    out = pl.pallas_call(
        kernel,
        out_shape=jax.ShapeDtypeStruct((B, D), A_x.dtype),
        in_specs=[pl.BlockSpec(memory_space=pl.ANY)] * 13,
        out_specs=pl.BlockSpec(memory_space=pltpu.VMEM),
        scratch_shapes=[
            pltpu.VMEM((B, D), bf16),
            pltpu.VMEM((B, D), bf16),
            pltpu.VMEM((F,), bf16),
            pltpu.VMEM((D,), bf16),
            pltpu.VMEM((D // _HM, _HM, HD + 6 * D), bf16),
            pltpu.VMEM((D // _W1M, _W1M, F), bf16),
            pltpu.VMEM((a_end, _MAJ, W), bf16),
            pltpu.VMEM((B, 6 * D), f32),
            pltpu.VMEM((B, D), bf16),
            pltpu.VMEM((W // 256, _HG, 256), f32),
            pltpu.VMEM((_HG, W), bf16),
            pltpu.VMEM((HD // 256, B, 256), f32),
            pltpu.SemaphoreType.DMA((sem_small + 4,)),
        ],
        compiler_params=pltpu.CompilerParams(
            vmem_limit_bytes=96 * 1024 * 1024,
            disable_bounds_checks=True,
            disable_semaphore_checks=True,
        ),
    )(A_x.reshape(B, D), *kv_views, A_wq.reshape(D // _HM, _HM, HD),
      A_wo.reshape(n_wo, _OM, D), B_w1.reshape(D // _W1M, _W1M, F), B_b1,
      B_w2.reshape(n_w2, _OM, D), B_b2, c, w_mod.reshape(D // _HM, _HM, 6 * D))
    return out.reshape(B, Sq, D)
```

```python
import functools

import jax
import jax.numpy as jnp
import jax.experimental.pallas as pl
import jax.experimental.pallas.tpu as pltpu

_EPS = 1e-05
_HG = 16
_MAJ = 64
_HM = 80
_OM = 384
_W1M = 160
_LAG = 25
_NVP = 10
_ORDER = (0, 3, 1, 2)


def _layernorm(x):
    m = jnp.mean(x, axis=-1, keepdims=True)
    d = x - m
    v = jnp.mean(d * d, axis=-1, keepdims=True)
    return d / jnp.sqrt(v + _EPS)


def _dot(a, b):
    return jnp.dot(a, b, preferred_element_type=jnp.float32)


def _dot_nt(a, b):
    return jax.lax.dot_general(a, b, (((1,), (1,)), ((), ())),
                               preferred_element_type=jnp.float32)


@jax.jit
def pallas_adaLN_cond__sliding_block_cached__mixer_channel_mlp__decode_kernel(
    A_x: jax.Array,
    A_k_cache: jax.Array,
    A_v_cache: jax.Array,
    A_wq: jax.Array,
    A_wo: jax.Array,
    B_x: jax.Array,
    B_w1: jax.Array,
    B_b1: jax.Array,
    B_w2: jax.Array,
    B_b2: jax.Array,
    c: jax.Array,
    w_mod: jax.Array,
):
    del B_x
    B, Sq, D = A_x.shape
    _, H, Sk, Dh = A_k_cache.shape
    F = B_w1.shape[1]
    W = min(4096, max(256, Sk // 4))
    HD = H * Dh
    assert (B, Sq, D, H, Dh, W, F) == (8, 1, 640, 32, 192, 1024, 1536)
    assert A_wq.shape == (D, HD)
    nh = H // _HG
    nblk = B * nh
    bm = _HG * Dh // _MAJ
    ns = bm // 2
    nbody = 8 * nblk
    n_wo, n_w2 = HD // _OM, F // _OM
    scale = Dh ** -0.5
    f32, bf16 = jnp.float32, jnp.bfloat16
    a_edge = 2 * 4 * ns
    a_q = a_edge + 2 * 4
    a_wo = a_q + nblk // 2
    a_w2 = a_wo + HD // 128
    a_end = a_w2 + F // 128
    sem_edge, sem_wm, sem_wq, sem_wo, sem_w1, sem_w2, sem_small = 4, 6, 7, 8, 11, 12, 16
    partial = functools.partial

    def kernel(x_hbm, k2_hbm, k6_hbm, v2_hbm, v6_hbm, wq_hbm, wo_hbm, w1_hbm, b1_hbm,
               w2_hbm, b2_hbm, c_hbm, wm_hbm, out_ref,
               x_v, c_v, b1_v, b2_v, wqm_v, w1_v, arena, mod_s, h_s, s_s, p_s, o_s, sem):
        kv_hbm = ({2: k2_hbm, 6: k6_hbm}, {2: v2_hbm, 6: v6_hbm})

        def aligned(v, n):
            return v if isinstance(v, int) else pl.multiple_of(v, n)

        def ring(arr, blk):
            return (4 * arr + (blk & 3)) * ns

        def kv_unit(arr, gb, t, q):
            blk = gb >> 3
            r8 = aligned((2 * (gb & 3) + t // 12) * 8, 8)
            octet, k = divmod(2 * (t % 12) + q, 4)
            a = _ORDER[k]
            m, g = 4 + 8 * octet + a, (a ^ 6) - a
            pltpu.make_async_copy(
                kv_hbm[arr][g].at[pl.ds(blk * (bm // g) + m // g, 2), m % g,
                                  pl.ds(r8, 8), pl.ds(Sk - W, W)],
                arena.at[ring(arr, blk) + 4 * octet + a, :, pl.ds(r8, 8), :],
                sem.at[2 * arr + (blk & 1)]).start(priority=q)

        def edge_unit(arr, o, r, q):
            m = nblk * bm - 4 + o if o < 4 else o - 4
            pltpu.make_async_copy(
                kv_hbm[arr][2].at[m // 2, m % 2, pl.ds(r, 16), pl.ds(Sk - W, W)],
                arena.at[a_edge + 4 * arr + (o if o < 4 else o ^ 6), o // 4, pl.ds(r, 16), :],
                sem.at[sem_edge + arr]).start(priority=q)

        def quad_unit(src, base, nmaj, s0, r, quad, q):
            pltpu.make_async_copy(
                src.at[pl.ds(4 * quad, 4), pl.ds(aligned(r * 8, 8), 8), :],
                arena.at[pl.ds(base + (r >> 4) * nmaj + 4 * quad, 4), (r >> 3) & 1,
                         pl.ds(aligned((r & 7) * 8, 8), 8), pl.ds(0, D)],
                sem.at[s0 + (r >> 4)]).start(priority=q)

        def wo_unit(s_even, s, q):
            u = 2 * s + q
            quad_unit(wo_hbm, a_wo, n_wo, sem_wo, (s_even >> 1) + u // 4, u % 4, q)

        def strip_unit(src, dst, col0, s, m, r, c0, w, q):
            pltpu.make_async_copy(src.at[m, pl.ds(r, 8), pl.ds(c0, w)],
                                  dst.at[m, pl.ds(r, 8), pl.ds(col0 + c0, w)],
                                  sem.at[s]).start(priority=q)

        def unit(gb, t, q, last=False):
            final_octet = 2 * (t % 12) + q >= ns - 4
            if isinstance(gb, int):
                kv_unit((gb >> 2) & 1, gb, t, q)
            elif last:
                if not final_octet:
                    pl.when(gb < nbody)(lambda: kv_unit(1, gb, t, q))
                pl.when(gb >= nbody)(lambda: wo_unit(ns * (gb - nbody), t, q))
            else:
                for arr in range(2):
                    go = (gb & 4) == 4 * arr
                    if final_octet:
                        go = jnp.logical_and(go, gb < nbody - 8)
                    pl.when(go)(partial(kv_unit, arr, gb, t, q))

        def pump(gb, t, last=False):
            unit(gb, t, 0, last)
            unit(gb + (t + _LAG) // ns, (t + _LAG) % ns, 1, last)

        def wait_all(ref, s):
            pltpu.make_async_copy(ref, ref, sem.at[s]).wait()

        c_cp, x_cp, b1_cp, b2_cp = (
            pltpu.make_async_copy(src, dst, sem.at[sem_small + i]) for i, (src, dst) in
            enumerate(((c_hbm, c_v), (x_hbm, x_v), (b1_hbm, b1_v), (b2_hbm, b2_v))))

        units = [partial(strip_unit, wm_hbm, wqm_v, HD, sem_wm, m, r, c0, 3 * D)
                 for r in range(0, _HM, 8) for c0 in (0, 3 * D) for m in range(D // _HM)]
        mod_step = len(units) // 2 + 12
        units += [partial(strip_unit, wq_hbm, wqm_v, 0, sem_wq,
                          *divmod(g // 3 * 8, _HM), g % 3 * 2048, 2048)
                  for g0 in range(16) for g in range(g0, D // 8 * 3, 16)]
        units += [partial(edge_unit, arr, o, r)
                  for r in range(0, _MAJ, 16) for arr in range(2) for o in range(8)]
        hi = units[0::2]
        lo = units[1::2] + [partial(unit, t // ns, t % ns) for t in range(_LAG)]

        for start in lo[:4]:
            start(1)
        for cp in (c_cp, x_cp, b1_cp, b2_cp):
            cp.start(priority=0)
        for start in lo[4:_LAG]:
            start(1)
        for t in range(len(hi)):
            hi[t](0)
            lo[t + _LAG](1)
            if t == 8:
                c_cp.wait()
                x_cp.wait()
                x = x_v[...].astype(f32)
                ln_x = _layernorm(x)
                sc = jax.nn.silu(c_v[...].astype(f32)).astype(bf16)
            if t == mod_step:
                wait_all(wqm_v.at[:, :, pl.ds(HD, 6 * D)], sem_wm)
            ct, odd = divmod(t - mod_step, 2)
            if 0 <= ct < 6 * D // 128 and not odd:
                w = wqm_v[:, :, pl.ds(HD + ct * 128, 128)].reshape(D, 128)
                mod_s[:, pl.ds(ct * 128, 128)] = _dot(sc, w)
                if ct == 2 * D // 128 + 1:
                    h_s[...] = (ln_x * (1.0 + mod_s[:, D:2 * D]) + mod_s[:, 0:D]).astype(bf16)

        for t in range(ns):
            pump(0, t)
        wait_all(wqm_v.at[:, :, pl.ds(0, HD)], sem_wq)
        for arr in range(2):
            wait_all(arena.at[pl.ds(a_edge + 4 * arr, 4)], sem_edge + arr)

        row1 = jax.lax.broadcasted_iota(jnp.int32, (_HG, 128), 0)
        col1 = jax.lax.broadcasted_iota(jnp.int32, (_HG, 128), 1)

        def q_tile(b, hf, kt):
            return arena.at[a_q + b, hf, pl.ds(aligned((kt >> 3) * _HG, _HG), _HG),
                            pl.ds(aligned((kt & 7) * 128, 128), 128)]

        def queries(i, carry):
            h = h_s[...]
            for t in range(12):
                pump(1 + i, 2 * t)
                c0 = pl.multiple_of((12 * i + t) * 128, 128)
                q = _dot(h, wqm_v[:, :, pl.ds(c0, 128)].reshape(D, 128))
                first = (row1 - 8 * (i & 1)) * Dh - 128 * t
                keep = jnp.logical_and(col1 >= first, col1 < first + Dh)
                for b in range(B):
                    if b == B // 2:
                        pump(1 + i, 2 * t + 1)
                    tile = jnp.where(keep, jnp.broadcast_to(q[b:b + 1, :], (_HG, 128)), 0.0)
                    q_tile(b, i >> 1, 12 * (i & 1) + t)[...] = tile.astype(bf16)
            return carry

        jax.lax.fori_loop(0, 4, queries, 0)

        row2 = jax.lax.broadcasted_iota(jnp.int32, (_HG, 256), 0)
        col2 = jax.lax.broadcasted_iota(jnp.int32, (_HG, 256), 1)

        def attend(n, last):
            def octets(arr):
                edge, before = a_edge + 4 * arr, ring(arr, n - 1) + ns - 4
                if last:
                    return before, ring(arr, n), edge
                return jnp.where(n == 0, edge, before), ring(arr, n), ring(arr, n) + ns - 4

            def rows128(cell, half, e, cols):
                tile = arena[pl.ds(cell + 2 * (e ^ half), 2), half, :, cols]
                return tile.reshape(2 * _MAJ, cols.size)

            k_before, k_block, k_final = octets(0)
            v_before, v_block, v_final = octets(1)

            def scores(i, carry):
                cols = pl.ds(pl.multiple_of(i * 256, 256), 256)
                acc = jnp.zeros((_HG, 256), f32)
                for t in range(ns):
                    pump(8 * n + 5 + i, t, last)
                    g = t // 2
                    cell = {0: k_before, 11: k_final}.get(g, k_block + 4 * ((g - 1) >> 1))
                    kt = rows128(cell, (g + 1) & 1, t & 1, cols)
                    acc = acc + _dot(q_tile(n >> 1, n & 1, t)[...], kt)
                s_s[i] = acc
                return carry

            def values(i, carry):
                for rp in range(3):
                    g = 3 * i + rp
                    cell = v_block + 4 * ((g - 1) >> 1)
                    if rp == 0:
                        cell = jnp.where(i == 0, v_before, cell)
                    if rp == 2:
                        cell = jnp.where(i == 3, v_final, cell)
                    acc = jnp.zeros((_HG, 256), f32)
                    for t in range(8):
                        z = rp * 8 + t
                        if not last:
                            pump(8 * n + 9 + i, z)
                        elif z * _NVP // ns != (z + 1) * _NVP // ns:
                            wo_unit(_NVP * i, ns + z * _NVP // ns, 0)
                            wo_unit(_NVP * i, ns + z * _NVP // ns + _LAG, 1)
                        cols = pl.ds(t * 128, 128)
                        vt = [rows128(cell, (g + 1) & 1, e, cols) for e in range(2)]
                        acc = acc + _dot_nt(p_s[:, cols], jnp.concatenate(vt, axis=0))
                    first = (row2 - 4 * i) * Dh - 256 * rp
                    keep = jnp.logical_and(col2 >= first, col2 < first + Dh)
                    o_s[(n & 1) * 12 + g, pl.ds(n >> 1, 1), :] = jnp.sum(
                        jnp.where(keep, acc, 0.0), axis=0, keepdims=True)
                return carry

            cells = ns - 4 if last else ns
            wait_all(arena.at[pl.ds(k_block, cells)], n & 1)
            jax.lax.fori_loop(0, 4, scores, 0)
            s = jnp.concatenate([s_s[t] for t in range(4)], axis=1) * scale
            p = jnp.exp(s - jnp.max(s, axis=-1, keepdims=True))
            p_s[...] = (p / jnp.sum(p, axis=-1, keepdims=True)).astype(bf16)
            wait_all(arena.at[pl.ds(v_block, cells)], 2 + (n & 1))
            jax.lax.fori_loop(0, 4, values, 0)

        def period(n, carry):
            attend(n, False)
            return carry

        jax.lax.fori_loop(0, nblk - 1, period, 0)
        attend(nblk - 1, True)

        w2_blocks = [
            pltpu.make_async_copy(w2_hbm.at[m, pl.ds((4 + e) * _MAJ, _MAJ), :],
                                  arena.at[a_w2 + 2 * n_w2 + m, e, :, pl.ds(0, D)],
                                  sem.at[sem_w2 + 2 + m // 3])
            for m in range(n_w2) for e in range(2)]
        units = [partial(quad_unit, wo_hbm, a_wo, n_wo, sem_wo, u // 4, u % 4)
                 for u in range(HD // 32)]
        w1_units = [partial(strip_unit, w1_hbm, w1_v, 0, sem_w1, m, r, 0, F)
                    for r in range(0, _W1M, 8) for m in range(D // _W1M)]
        w2_units = [partial(quad_unit, w2_hbm, a_w2, n_w2, sem_w2, r, 0) for r in range(32)]
        for r in range(16):
            units += w1_units[5 * r:5 * r + 5] + [w2_units[r]]
        hi = units[0::2]
        lo = units[1::2] + w2_units[16:] + [cp.start for cp in w2_blocks]
        assert len(lo) <= len(hi) + _LAG

        def w_cells(cell, n):
            return arena.at[pl.ds(cell, n), :, :, pl.ds(0, D)]

        s0 = ns + 4 * _NVP
        chunk_step = (s0, s0 + n_wo, HD // 64 + 8)
        attn = jnp.zeros((B, D), f32)
        for t in range(s0, len(hi)):
            if t in chunk_step:
                c3 = chunk_step.index(t)
                wait_all(w_cells(a_wo + n_wo * c3, n_wo), sem_wo + c3)
            hi[t](0)
            if t + _LAG < len(lo):
                lo[t + _LAG](1)
            m = t - chunk_step[c3]
            if m < n_wo:
                col = m * _OM + c3 * 128
                o_t = o_s[col // 256, :, pl.ds(col % 256, 128)].astype(bf16)
                attn = attn + _dot(o_t, w_cells(a_wo + n_wo * c3 + m, 1)[...].reshape(128, D))
            if (c3, m) == (2, n_wo - 1):
                ga, sb, cb, gb = (mod_s[:, k * D:(k + 1) * D] for k in range(2, 6))
                x1 = x + ga * attn
                h2 = _layernorm(x1) * (1.0 + cb) + sb
                y = _layernorm(h2).astype(bf16)

        b1_cp.wait()
        b2_cp.wait()
        wait_all(w1_v, sem_w1)
        u = _dot(y, w1_v[...].reshape(D, F)) + b1_v[...].astype(f32).reshape(1, F)
        u = jax.nn.gelu(u, approximate=True).astype(bf16)

        def w2_dot(k0, k1):
            cols = [k % n_w2 * _OM + k // n_w2 * 128 for k in range(k0, k1)]
            lhs = jnp.concatenate([u[:, j:j + 128] for j in cols], axis=1)
            return _dot(lhs, w_cells(a_w2 + k0, k1 - k0)[...].reshape(128 * (k1 - k0), D))

        for c3 in range(2):
            wait_all(w_cells(a_w2 + n_w2 * c3, n_w2), sem_w2 + c3)
        mlp = b2_v[...].astype(f32).reshape(1, D) + w2_dot(0, 8)
        for cp in w2_blocks[:6]:
            cp.wait()
        mlp = mlp + w2_dot(8, 11)
        for cp in w2_blocks[6:]:
            cp.wait()
        mlp = mlp + w2_dot(11, 12)
        out_ref[...] = (x1 + gb * mlp).astype(out_ref.dtype)

    kv_views = [jnp.swapaxes(a, 2, 3).reshape(nblk * bm // g, g, _MAJ, Sk)
                for a in (A_k_cache, A_v_cache) for g in (2, 6)]

    out = pl.pallas_call(
        kernel,
        out_shape=jax.ShapeDtypeStruct((B, D), A_x.dtype),
        in_specs=[pl.BlockSpec(memory_space=pl.ANY)] * 13,
        out_specs=pl.BlockSpec(memory_space=pltpu.VMEM),
        scratch_shapes=[
            pltpu.VMEM((B, D), bf16),
            pltpu.VMEM((B, D), bf16),
            pltpu.VMEM((F,), bf16),
            pltpu.VMEM((D,), bf16),
            pltpu.VMEM((D // _HM, _HM, HD + 6 * D), bf16),
            pltpu.VMEM((D // _W1M, _W1M, F), bf16),
            pltpu.VMEM((a_end, 2, _MAJ, W), bf16),
            pltpu.VMEM((B, 6 * D), f32),
            pltpu.VMEM((B, D), bf16),
            pltpu.VMEM((W // 256, _HG, 256), f32),
            pltpu.VMEM((_HG, W), bf16),
            pltpu.VMEM((HD // 256, B, 256), f32),
            pltpu.SemaphoreType.DMA((sem_small + 4,)),
        ],
        compiler_params=pltpu.CompilerParams(
            vmem_limit_bytes=100 * 1024 * 1024,
            disable_bounds_checks=True,
            disable_semaphore_checks=True,
        ),
    )(A_x.reshape(B, D), *kv_views, A_wq.reshape(D // _HM, _HM, HD),
      A_wo.reshape(n_wo, _OM, D), B_w1.reshape(D // _W1M, _W1M, F), B_b1,
      B_w2.reshape(n_w2, _OM, D), B_b2, c, w_mod.reshape(D // _HM, _HM, 6 * D))
    return out.reshape(B, Sq, D)
```

```python
import functools

import jax
import jax.numpy as jnp
import jax.experimental.pallas as pl
import jax.experimental.pallas.tpu as pltpu

_EPS = 1e-05
_HG = 16
_MAJ = 64
_HM = 80
_OM = 384
_W1M = 160
_LAG = 25
_NVP = 10
_W2_STAGES = (8, 10, 11, 12)
_ORDER = (0, 3, 1, 2)


def _layernorm(x):
    m = jnp.mean(x, axis=-1, keepdims=True)
    d = x - m
    v = jnp.mean(d * d, axis=-1, keepdims=True)
    return d / jnp.sqrt(v + _EPS)


def _dot(a, b):
    return jnp.dot(a, b, preferred_element_type=jnp.float32)


def _dot_nt(a, b):
    return jax.lax.dot_general(a, b, (((1,), (1,)), ((), ())),
                               preferred_element_type=jnp.float32)


@jax.jit
def pallas_adaLN_cond__sliding_block_cached__mixer_channel_mlp__decode_kernel(
    A_x: jax.Array,
    A_k_cache: jax.Array,
    A_v_cache: jax.Array,
    A_wq: jax.Array,
    A_wo: jax.Array,
    B_x: jax.Array,
    B_w1: jax.Array,
    B_b1: jax.Array,
    B_w2: jax.Array,
    B_b2: jax.Array,
    c: jax.Array,
    w_mod: jax.Array,
):
    del B_x
    B, Sq, D = A_x.shape
    _, H, Sk, Dh = A_k_cache.shape
    F = B_w1.shape[1]
    W = min(4096, max(256, Sk // 4))
    HD = H * Dh
    assert (B, Sq, D, H, Dh, W, F) == (8, 1, 640, 32, 192, 1024, 1536)
    assert A_wq.shape == (D, HD)
    nh = H // _HG
    nblk = B * nh
    bm = _HG * Dh // _MAJ
    ns = bm // 2
    nbody = 8 * nblk
    n_wo, n_w2 = HD // _OM, F // _OM
    scale = Dh ** -0.5
    f32, bf16 = jnp.float32, jnp.bfloat16
    a_edge = 2 * 4 * ns
    a_q = a_edge + 2 * 4
    a_wo = a_q + nblk // 2
    a_w2 = a_wo + HD // 128
    a_end = a_w2 + F // 128
    sem_edge, sem_wm, sem_wq, sem_wo, sem_w1, sem_w2, sem_small = 4, 6, 7, 8, 11, 12, 17
    partial = functools.partial

    def kernel(x_hbm, k2_hbm, k6_hbm, v2_hbm, v6_hbm, wq_hbm, wo_hbm, w1_hbm, b1_hbm,
               w2_hbm, b2_hbm, c_hbm, wm_hbm, out_ref,
               x_v, c_v, b1_v, b2_v, wqm_v, w1_v, arena, mod_s, h_s, s_s, p_s, o_s, sem):
        kv_hbm = ({2: k2_hbm, 6: k6_hbm}, {2: v2_hbm, 6: v6_hbm})

        def aligned(v, n):
            return v if isinstance(v, int) else pl.multiple_of(v, n)

        def ring(arr, blk):
            return (4 * arr + (blk & 3)) * ns

        def kv_unit(arr, gb, t, q):
            blk = gb >> 3
            r8 = aligned((2 * (gb & 3) + t // 12) * 8, 8)
            octet, k = divmod(2 * (t % 12) + q, 4)
            a = _ORDER[k]
            m, g = 4 + 8 * octet + a, (a ^ 6) - a
            pltpu.make_async_copy(
                kv_hbm[arr][g].at[pl.ds(blk * (bm // g) + m // g, 2), m % g,
                                  pl.ds(r8, 8), pl.ds(Sk - W, W)],
                arena.at[ring(arr, blk) + 4 * octet + a, :, pl.ds(r8, 8), :],
                sem.at[2 * arr + (blk & 1)]).start(priority=q)

        def edge_unit(arr, o, r, q):
            m = nblk * bm - 4 + o if o < 4 else o - 4
            pltpu.make_async_copy(
                kv_hbm[arr][2].at[m // 2, m % 2, pl.ds(r, 16), pl.ds(Sk - W, W)],
                arena.at[a_edge + 4 * arr + (o if o < 4 else o ^ 6), o // 4, pl.ds(r, 16), :],
                sem.at[sem_edge + arr]).start(priority=q)

        def quad_unit(src, base, nmaj, s0, r, quad, q):
            pltpu.make_async_copy(
                src.at[pl.ds(4 * quad, 4), pl.ds(aligned(r * 8, 8), 8), :],
                arena.at[pl.ds(base + (r >> 4) * nmaj + 4 * quad, 4), (r >> 3) & 1,
                         pl.ds(aligned((r & 7) * 8, 8), 8), pl.ds(0, D)],
                sem.at[s0 + (r >> 4)]).start(priority=q)

        def wo_unit(s_even, s, q):
            u = 2 * s + q
            quad_unit(wo_hbm, a_wo, n_wo, sem_wo, (s_even >> 1) + u // 4, u % 4, q)

        def strip_unit(src, dst, col0, s, m, r, c0, w, q):
            pltpu.make_async_copy(src.at[m, pl.ds(r, 8), pl.ds(c0, w)],
                                  dst.at[m, pl.ds(r, 8), pl.ds(col0 + c0, w)],
                                  sem.at[s]).start(priority=q)

        def unit(gb, t, q, last=False):
            final_octet = 2 * (t % 12) + q >= ns - 4
            if isinstance(gb, int):
                kv_unit((gb >> 2) & 1, gb, t, q)
            elif last:
                if not final_octet:
                    pl.when(gb < nbody)(lambda: kv_unit(1, gb, t, q))
                pl.when(gb >= nbody)(lambda: wo_unit(ns * (gb - nbody), t, q))
            else:
                for arr in range(2):
                    go = (gb & 4) == 4 * arr
                    if final_octet:
                        go = jnp.logical_and(go, gb < nbody - 8)
                    pl.when(go)(partial(kv_unit, arr, gb, t, q))

        def pump(gb, t, last=False):
            unit(gb, t, 0, last)
            unit(gb + (t + _LAG) // ns, (t + _LAG) % ns, 1, last)

        def wait_all(ref, s):
            pltpu.make_async_copy(ref, ref, sem.at[s]).wait()

        c_cp, x_cp, b1_cp, b2_cp = (
            pltpu.make_async_copy(src, dst, sem.at[sem_small + i]) for i, (src, dst) in
            enumerate(((c_hbm, c_v), (x_hbm, x_v), (b1_hbm, b1_v), (b2_hbm, b2_v))))

        units = [partial(strip_unit, wm_hbm, wqm_v, HD, sem_wm, m, r, c0, 3 * D)
                 for r in range(0, _HM, 8) for c0 in (0, 3 * D) for m in range(D // _HM)]
        mod_step = len(units) // 2 + 12
        units += [partial(strip_unit, wq_hbm, wqm_v, 0, sem_wq,
                          *divmod(g // 3 * 8, _HM), g % 3 * 2048, 2048)
                  for g0 in range(16) for g in range(g0, D // 8 * 3, 16)]
        units += [partial(edge_unit, arr, o, r)
                  for r in range(0, _MAJ, 16) for arr in range(2) for o in range(8)]
        hi = units[0::2]
        lo = units[1::2] + [partial(unit, t // ns, t % ns) for t in range(_LAG)]

        for start in lo[:4]:
            start(1)
        for cp in (c_cp, x_cp, b1_cp, b2_cp):
            cp.start(priority=0)
        for start in lo[4:_LAG]:
            start(1)
        for t in range(len(hi)):
            hi[t](0)
            lo[t + _LAG](1)
            if t == 8:
                c_cp.wait()
                x_cp.wait()
                x = x_v[...].astype(f32)
                ln_x = _layernorm(x)
                sc = jax.nn.silu(c_v[...].astype(f32)).astype(bf16)
            if t == mod_step:
                wait_all(wqm_v.at[:, :, pl.ds(HD, 6 * D)], sem_wm)
            ct, odd = divmod(t - mod_step, 2)
            if 0 <= ct < 6 * D // 128 and not odd:
                w = wqm_v[:, :, pl.ds(HD + ct * 128, 128)].reshape(D, 128)
                mod_s[:, pl.ds(ct * 128, 128)] = _dot(sc, w)
                if ct == 2 * D // 128 + 1:
                    h_s[...] = (ln_x * (1.0 + mod_s[:, D:2 * D]) + mod_s[:, 0:D]).astype(bf16)

        for t in range(ns):
            pump(0, t)
        wait_all(wqm_v.at[:, :, pl.ds(0, HD)], sem_wq)
        for arr in range(2):
            wait_all(arena.at[pl.ds(a_edge + 4 * arr, 4)], sem_edge + arr)

        row1 = jax.lax.broadcasted_iota(jnp.int32, (_HG, 128), 0)
        col1 = jax.lax.broadcasted_iota(jnp.int32, (_HG, 128), 1)

        def q_tile(b, hf, kt):
            return arena.at[a_q + b, hf, pl.ds(aligned((kt >> 3) * _HG, _HG), _HG),
                            pl.ds(aligned((kt & 7) * 128, 128), 128)]

        def queries(i, carry):
            h = h_s[...]
            for t in range(12):
                pump(1 + i, 2 * t)
                c0 = pl.multiple_of((12 * i + t) * 128, 128)
                q = _dot(h, wqm_v[:, :, pl.ds(c0, 128)].reshape(D, 128))
                first = (row1 - 8 * (i & 1)) * Dh - 128 * t
                keep = jnp.logical_and(col1 >= first, col1 < first + Dh)
                for b in range(B):
                    if b == B // 2:
                        pump(1 + i, 2 * t + 1)
                    tile = jnp.where(keep, jnp.broadcast_to(q[b:b + 1, :], (_HG, 128)), 0.0)
                    q_tile(b, i >> 1, 12 * (i & 1) + t)[...] = tile.astype(bf16)
            return carry

        jax.lax.fori_loop(0, 4, queries, 0)

        row2 = jax.lax.broadcasted_iota(jnp.int32, (_HG, 256), 0)
        col2 = jax.lax.broadcasted_iota(jnp.int32, (_HG, 256), 1)

        def attend(n, last):
            def octets(arr):
                edge, before = a_edge + 4 * arr, ring(arr, n - 1) + ns - 4
                if last:
                    return before, ring(arr, n), edge
                return jnp.where(n == 0, edge, before), ring(arr, n), ring(arr, n) + ns - 4

            def rows128(cell, half, e, cols):
                tile = arena[pl.ds(cell + 2 * (e ^ half), 2), half, :, cols]
                return tile.reshape(2 * _MAJ, cols.size)

            k_before, k_block, k_final = octets(0)
            v_before, v_block, v_final = octets(1)

            def scores(i, carry):
                cols = pl.ds(pl.multiple_of(i * 256, 256), 256)
                acc = jnp.zeros((_HG, 256), f32)
                for t in range(ns):
                    pump(8 * n + 5 + i, t, last)
                    g = t // 2
                    cell = {0: k_before, 11: k_final}.get(g, k_block + 4 * ((g - 1) >> 1))
                    kt = rows128(cell, (g + 1) & 1, t & 1, cols)
                    acc = acc + _dot(q_tile(n >> 1, n & 1, t)[...], kt)
                s_s[i] = acc
                return carry

            def values(i, carry):
                for rp in range(3):
                    g = 3 * i + rp
                    cell = v_block + 4 * ((g - 1) >> 1)
                    if rp == 0:
                        cell = jnp.where(i == 0, v_before, cell)
                    if rp == 2:
                        cell = jnp.where(i == 3, v_final, cell)
                    acc = jnp.zeros((_HG, 256), f32)
                    for t in range(8):
                        z = rp * 8 + t
                        if not last:
                            pump(8 * n + 9 + i, z)
                        elif z * _NVP // ns != (z + 1) * _NVP // ns:
                            wo_unit(_NVP * i, ns + z * _NVP // ns, 0)
                            wo_unit(_NVP * i, ns + z * _NVP // ns + _LAG, 1)
                        cols = pl.ds(t * 128, 128)
                        vt = [rows128(cell, (g + 1) & 1, e, cols) for e in range(2)]
                        acc = acc + _dot_nt(p_s[:, cols], jnp.concatenate(vt, axis=0))
                    first = (row2 - 4 * i) * Dh - 256 * rp
                    keep = jnp.logical_and(col2 >= first, col2 < first + Dh)
                    o_s[(n & 1) * 12 + g, pl.ds(n >> 1, 1), :] = jnp.sum(
                        jnp.where(keep, acc, 0.0), axis=0, keepdims=True)
                return carry

            cells = ns - 4 if last else ns
            wait_all(arena.at[pl.ds(k_block, cells)], n & 1)
            jax.lax.fori_loop(0, 4, scores, 0)
            s = jnp.concatenate([s_s[t] for t in range(4)], axis=1) * scale
            p = jnp.exp(s - jnp.max(s, axis=-1, keepdims=True))
            p_s[...] = (p / jnp.sum(p, axis=-1, keepdims=True)).astype(bf16)
            wait_all(arena.at[pl.ds(v_block, cells)], 2 + (n & 1))
            jax.lax.fori_loop(0, 4, values, 0)

        def period(n, carry):
            attend(n, False)
            return carry

        jax.lax.fori_loop(0, nblk - 1, period, 0)
        attend(nblk - 1, True)

        def w2_piece(m, e, q):
            stage = [2 * n_w2 + m < k for k in _W2_STAGES].index(True)
            pltpu.make_async_copy(w2_hbm.at[m, pl.ds((4 + e) * _MAJ, _MAJ), :],
                                  arena.at[a_w2 + 2 * n_w2 + m, e, :, pl.ds(0, D)],
                                  sem.at[sem_w2 + 1 + stage]).start(priority=q)

        units = [partial(quad_unit, wo_hbm, a_wo, n_wo, sem_wo, u // 4, u % 4)
                 for u in range(HD // 32)]
        w1_units = [partial(strip_unit, w1_hbm, w1_v, 0, sem_w1, m, r, 0, F)
                    for r in range(0, _W1M, 8) for m in range(D // _W1M)]
        w2_units = [partial(quad_unit, w2_hbm, a_w2, n_w2, sem_w2, r, 0) for r in range(32)]
        for r in range(16):
            units += w1_units[5 * r:5 * r + 5] + [w2_units[r]]
        hi = units[0::2]
        lo = units[1::2] + w2_units[16:] + [
            partial(w2_piece, m, e) for m in range(n_w2) for e in range(2)]
        assert len(lo) <= len(hi) + _LAG

        def w_cells(cell, n):
            return arena.at[pl.ds(cell, n), :, :, pl.ds(0, D)]

        s0 = ns + 4 * _NVP
        chunk_step = (s0, s0 + n_wo, HD // 64 + 8)
        attn = jnp.zeros((B, D), f32)
        for t in range(s0, len(hi)):
            if t in chunk_step:
                c3 = chunk_step.index(t)
                wait_all(w_cells(a_wo + n_wo * c3, n_wo), sem_wo + c3)
            hi[t](0)
            if t + _LAG < len(lo):
                lo[t + _LAG](1)
            m = t - chunk_step[c3]
            if m < n_wo:
                col = m * _OM + c3 * 128
                o_t = o_s[col // 256, :, pl.ds(col % 256, 128)].astype(bf16)
                attn = attn + _dot(o_t, w_cells(a_wo + n_wo * c3 + m, 1)[...].reshape(128, D))
            if (c3, m) == (2, n_wo - 1):
                ga, sb, cb, gb = (mod_s[:, k * D:(k + 1) * D] for k in range(2, 6))
                x1 = x + ga * attn
                h2 = _layernorm(x1) * (1.0 + cb) + sb
                y = _layernorm(h2).astype(bf16)

        b1_cp.wait()
        b2_cp.wait()
        wait_all(w1_v, sem_w1)
        u = _dot(y, w1_v[...].reshape(D, F)) + b1_v[...].astype(f32).reshape(1, F)
        u = jax.nn.gelu(u, approximate=True).astype(bf16)

        def w2_dot(k0, k1):
            cols = [k % n_w2 * _OM + k // n_w2 * 128 for k in range(k0, k1)]
            lhs = jnp.concatenate([u[:, j:j + 128] for j in cols], axis=1)
            return _dot(lhs, w_cells(a_w2 + k0, k1 - k0)[...].reshape(128 * (k1 - k0), D))

        for c3 in range(2):
            wait_all(w_cells(a_w2 + n_w2 * c3, n_w2), sem_w2 + c3)
        mlp = b2_v[...].astype(f32).reshape(1, D) + w2_dot(0, _W2_STAGES[0])
        for stage, (k0, k1) in enumerate(zip(_W2_STAGES, _W2_STAGES[1:])):
            wait_all(w_cells(a_w2 + k0, k1 - k0), sem_w2 + 2 + stage)
            mlp = mlp + w2_dot(k0, k1)
        out_ref[...] = (x1 + gb * mlp).astype(out_ref.dtype)

    kv_views = [jnp.swapaxes(a, 2, 3).reshape(nblk * bm // g, g, _MAJ, Sk)
                for a in (A_k_cache, A_v_cache) for g in (2, 6)]

    out = pl.pallas_call(
        kernel,
        out_shape=jax.ShapeDtypeStruct((B, D), A_x.dtype),
        in_specs=[pl.BlockSpec(memory_space=pl.ANY)] * 13,
        out_specs=pl.BlockSpec(memory_space=pltpu.VMEM),
        scratch_shapes=[
            pltpu.VMEM((B, D), bf16),
            pltpu.VMEM((B, D), bf16),
            pltpu.VMEM((F,), bf16),
            pltpu.VMEM((D,), bf16),
            pltpu.VMEM((D // _HM, _HM, HD + 6 * D), bf16),
            pltpu.VMEM((D // _W1M, _W1M, F), bf16),
            pltpu.VMEM((a_end, 2, _MAJ, W), bf16),
            pltpu.VMEM((B, 6 * D), f32),
            pltpu.VMEM((B, D), bf16),
            pltpu.VMEM((W // 256, _HG, 256), f32),
            pltpu.VMEM((_HG, W), bf16),
            pltpu.VMEM((HD // 256, B, 256), f32),
            pltpu.SemaphoreType.DMA((sem_small + 4,)),
        ],
        compiler_params=pltpu.CompilerParams(
            vmem_limit_bytes=100 * 1024 * 1024,
            disable_bounds_checks=True,
            disable_semaphore_checks=True,
        ),
    )(A_x.reshape(B, D), *kv_views, A_wq.reshape(D // _HM, _HM, HD),
      A_wo.reshape(n_wo, _OM, D), B_w1.reshape(D // _W1M, _W1M, F), B_b1,
      B_w2.reshape(n_w2, _OM, D), B_b2, c, w_mod.reshape(D // _HM, _HM, 6 * D))
    return out.reshape(B, Sq, D)
```

```python
import functools

import jax
import jax.numpy as jnp
import jax.experimental.pallas as pl
import jax.experimental.pallas.tpu as pltpu

_EPS = 1e-05
_HG = 16
_MAJ = 64
_HM = 80
_OM = 384
_W1M = 160
_LAG = 25
_NVP = 10
_W2_STAGES = (8, 10, 11, 12)
_ORDER = (0, 3, 1, 2)


def _layernorm(x):
    m = jnp.mean(x, axis=-1, keepdims=True)
    d = x - m
    v = jnp.mean(d * d, axis=-1, keepdims=True)
    return d / jnp.sqrt(v + _EPS)


def _dot(a, b):
    return jnp.dot(a, b, preferred_element_type=jnp.float32)


def _dot_nt(a, b):
    return jax.lax.dot_general(a, b, (((1,), (1,)), ((), ())),
                               preferred_element_type=jnp.float32)


@jax.jit
def pallas_adaLN_cond__sliding_block_cached__mixer_channel_mlp__decode_kernel(
    A_x: jax.Array,
    A_k_cache: jax.Array,
    A_v_cache: jax.Array,
    A_wq: jax.Array,
    A_wo: jax.Array,
    B_x: jax.Array,
    B_w1: jax.Array,
    B_b1: jax.Array,
    B_w2: jax.Array,
    B_b2: jax.Array,
    c: jax.Array,
    w_mod: jax.Array,
):
    del B_x
    B, Sq, D = A_x.shape
    _, H, Sk, Dh = A_k_cache.shape
    F = B_w1.shape[1]
    W = min(4096, max(256, Sk // 4))
    HD = H * Dh
    assert (B, Sq, D, H, Dh, W, F) == (8, 1, 640, 32, 192, 1024, 1536)
    assert A_wq.shape == (D, HD)
    nh = H // _HG
    nblk = B * nh
    bm = _HG * Dh // _MAJ
    ns = bm // 2
    nbody = 8 * nblk
    n_wo, n_w2 = HD // _OM, F // _OM
    scale = Dh ** -0.5
    f32, bf16 = jnp.float32, jnp.bfloat16
    a_edge = 2 * 4 * ns
    a_q = a_edge + 2 * 4
    a_wo = a_q + nblk // 2
    a_w2 = a_wo + HD // 128
    a_end = a_w2 + F // 128
    sem_edge, sem_wm, sem_wq, sem_wo, sem_w1, sem_w2, sem_small = 4, 6, 7, 8, 11, 12, 17
    partial = functools.partial

    def kernel(x_hbm, k2_hbm, k6_hbm, v2_hbm, v6_hbm, wq_hbm, wo_hbm, w1_hbm, b1_hbm,
               w2_hbm, b2_hbm, c_hbm, wm_hbm, out_ref,
               x_v, c_v, b1_v, b2_v, wqm_v, w1_v, arena, mod_s, h_s, s_s, p_s, o_s, sem):
        kv_hbm = ({2: k2_hbm, 6: k6_hbm}, {2: v2_hbm, 6: v6_hbm})

        def aligned(v, n):
            return v if isinstance(v, int) else pl.multiple_of(v, n)

        def ring(arr, blk):
            return (4 * arr + (blk & 3)) * ns

        def kv_unit(arr, gb, t, q):
            blk = gb >> 3
            r8 = aligned((2 * (gb & 3) + t // 12) * 8, 8)
            octet, k = divmod(2 * (t % 12) + q, 4)
            a = _ORDER[k]
            m, g = 4 + 8 * octet + a, (a ^ 6) - a
            pltpu.make_async_copy(
                kv_hbm[arr][g].at[pl.ds(blk * (bm // g) + m // g, 2), m % g,
                                  pl.ds(r8, 8), pl.ds(Sk - W, W)],
                arena.at[ring(arr, blk) + 4 * octet + a, :, pl.ds(r8, 8), :],
                sem.at[2 * arr + (blk & 1)]).start(priority=q)

        def edge_unit(arr, o, r, q):
            m = nblk * bm - 4 + o if o < 4 else o - 4
            cell = a_edge + 4 * arr + (o if o < 4 else o ^ 6)
            pltpu.make_async_copy(
                kv_hbm[arr][2].at[m // 2, :, pl.ds(r, 8), pl.ds(Sk - W, W)],
                arena.at[pl.ds(cell, 2), o // 4, pl.ds(r, 8), :],
                sem.at[sem_edge + arr]).start(priority=q)

        def quad_unit(src, base, nmaj, s0, r, quad, q):
            pltpu.make_async_copy(
                src.at[pl.ds(4 * quad, 4), pl.ds(aligned(r * 8, 8), 8), :],
                arena.at[pl.ds(base + (r >> 4) * nmaj + 4 * quad, 4), (r >> 3) & 1,
                         pl.ds(aligned((r & 7) * 8, 8), 8), pl.ds(0, D)],
                sem.at[s0 + (r >> 4)]).start(priority=q)

        def wo_unit(s_even, s, q):
            u = 2 * s + q
            quad_unit(wo_hbm, a_wo, n_wo, sem_wo, (s_even >> 1) + u // 4, u % 4, q)

        def strip_unit(src, dst, col0, s, m, r, c0, w, q):
            pltpu.make_async_copy(src.at[m, pl.ds(r, 8), pl.ds(c0, w)],
                                  dst.at[m, pl.ds(r, 8), pl.ds(col0 + c0, w)],
                                  sem.at[s]).start(priority=q)

        def unit(gb, t, q, last=False):
            final_octet = 2 * (t % 12) + q >= ns - 4
            if isinstance(gb, int):
                kv_unit((gb >> 2) & 1, gb, t, q)
            elif last:
                if not final_octet:
                    pl.when(gb < nbody)(lambda: kv_unit(1, gb, t, q))
                pl.when(gb >= nbody)(lambda: wo_unit(ns * (gb - nbody), t, q))
            else:
                for arr in range(2):
                    go = (gb & 4) == 4 * arr
                    if final_octet:
                        go = jnp.logical_and(go, gb < nbody - 8)
                    pl.when(go)(partial(kv_unit, arr, gb, t, q))

        def pump(gb, t, last=False):
            unit(gb, t, 0, last)
            unit(gb + (t + _LAG) // ns, (t + _LAG) % ns, 1, last)

        def wait_all(ref, s):
            pltpu.make_async_copy(ref, ref, sem.at[s]).wait()

        c_cp, x_cp, b1_cp, b2_cp = (
            pltpu.make_async_copy(src, dst, sem.at[sem_small + i]) for i, (src, dst) in
            enumerate(((c_hbm, c_v), (x_hbm, x_v), (b1_hbm, b1_v), (b2_hbm, b2_v))))

        units = [partial(strip_unit, wm_hbm, wqm_v, HD, sem_wm, m, r, c0, 3 * D)
                 for r in range(0, _HM, 8) for c0 in (0, 3 * D) for m in range(D // _HM)]
        mod_step = len(units) // 2 + 12
        units += [partial(strip_unit, wq_hbm, wqm_v, 0, sem_wq,
                          *divmod(g // 3 * 8, _HM), g % 3 * 2048, 2048)
                  for g0 in range(16) for g in range(g0, D // 8 * 3, 16)]
        units += [partial(edge_unit, arr, o, r)
                  for r in range(0, _MAJ, 8) for arr in range(2) for o in range(0, 8, 2)]
        hi = units[0::2]
        lo = units[1::2] + [partial(unit, t // ns, t % ns) for t in range(_LAG)]

        for start in lo[:4]:
            start(1)
        for cp in (c_cp, x_cp, b1_cp, b2_cp):
            cp.start(priority=0)
        for start in lo[4:_LAG]:
            start(1)
        for t in range(len(hi)):
            hi[t](0)
            lo[t + _LAG](1)
            if t == 8:
                c_cp.wait()
                x_cp.wait()
                x = x_v[...].astype(f32)
                ln_x = _layernorm(x)
                sc = jax.nn.silu(c_v[...].astype(f32)).astype(bf16)
            if t == mod_step:
                wait_all(wqm_v.at[:, :, pl.ds(HD, 6 * D)], sem_wm)
            ct, odd = divmod(t - mod_step, 2)
            if 0 <= ct < 6 * D // 128 and not odd:
                w = wqm_v[:, :, pl.ds(HD + ct * 128, 128)].reshape(D, 128)
                mod_s[:, pl.ds(ct * 128, 128)] = _dot(sc, w)
                if ct == 2 * D // 128 + 1:
                    h_s[...] = (ln_x * (1.0 + mod_s[:, D:2 * D]) + mod_s[:, 0:D]).astype(bf16)

        for t in range(ns):
            pump(0, t)
        wait_all(wqm_v.at[:, :, pl.ds(0, HD)], sem_wq)
        for arr in range(2):
            wait_all(arena.at[pl.ds(a_edge + 4 * arr, 4)], sem_edge + arr)

        row1 = jax.lax.broadcasted_iota(jnp.int32, (_HG, 128), 0)
        col1 = jax.lax.broadcasted_iota(jnp.int32, (_HG, 128), 1)

        def q_tile(b, hf, kt):
            return arena.at[a_q + b, hf, pl.ds(aligned((kt >> 3) * _HG, _HG), _HG),
                            pl.ds(aligned((kt & 7) * 128, 128), 128)]

        def queries(i, carry):
            h = h_s[...]
            for t in range(12):
                pump(1 + i, 2 * t)
                c0 = pl.multiple_of((12 * i + t) * 128, 128)
                q = _dot(h, wqm_v[:, :, pl.ds(c0, 128)].reshape(D, 128))
                first = (row1 - 8 * (i & 1)) * Dh - 128 * t
                keep = jnp.logical_and(col1 >= first, col1 < first + Dh)
                for b in range(B):
                    if b == B // 2:
                        pump(1 + i, 2 * t + 1)
                    tile = jnp.where(keep, jnp.broadcast_to(q[b:b + 1, :], (_HG, 128)), 0.0)
                    q_tile(b, i >> 1, 12 * (i & 1) + t)[...] = tile.astype(bf16)
            return carry

        jax.lax.fori_loop(0, 4, queries, 0)

        row2 = jax.lax.broadcasted_iota(jnp.int32, (_HG, 256), 0)
        col2 = jax.lax.broadcasted_iota(jnp.int32, (_HG, 256), 1)

        def attend(n, last):
            def octets(arr):
                edge, before = a_edge + 4 * arr, ring(arr, n - 1) + ns - 4
                if last:
                    return before, ring(arr, n), edge
                return jnp.where(n == 0, edge, before), ring(arr, n), ring(arr, n) + ns - 4

            def rows128(cell, half, e, cols):
                tile = arena[pl.ds(cell + 2 * (e ^ half), 2), half, :, cols]
                return tile.reshape(2 * _MAJ, cols.size)

            k_before, k_block, k_final = octets(0)
            v_before, v_block, v_final = octets(1)

            def scores(i, carry):
                cols = pl.ds(pl.multiple_of(i * 256, 256), 256)
                acc = jnp.zeros((_HG, 256), f32)
                for t in range(ns):
                    pump(8 * n + 5 + i, t, last)
                    g = t // 2
                    cell = {0: k_before, 11: k_final}.get(g, k_block + 4 * ((g - 1) >> 1))
                    kt = rows128(cell, (g + 1) & 1, t & 1, cols)
                    acc = acc + _dot(q_tile(n >> 1, n & 1, t)[...], kt)
                s_s[i] = acc
                return carry

            def values(i, carry):
                for rp in range(3):
                    g = 3 * i + rp
                    cell = v_block + 4 * ((g - 1) >> 1)
                    if rp == 0:
                        cell = jnp.where(i == 0, v_before, cell)
                    if rp == 2:
                        cell = jnp.where(i == 3, v_final, cell)
                    acc = jnp.zeros((_HG, 256), f32)
                    for t in range(8):
                        z = rp * 8 + t
                        if not last:
                            pump(8 * n + 9 + i, z)
                        elif z * _NVP // ns != (z + 1) * _NVP // ns:
                            wo_unit(_NVP * i, ns + z * _NVP // ns, 0)
                            wo_unit(_NVP * i, ns + z * _NVP // ns + _LAG, 1)
                        cols = pl.ds(t * 128, 128)
                        vt = [rows128(cell, (g + 1) & 1, e, cols) for e in range(2)]
                        acc = acc + _dot_nt(p_s[:, cols], jnp.concatenate(vt, axis=0))
                    first = (row2 - 4 * i) * Dh - 256 * rp
                    keep = jnp.logical_and(col2 >= first, col2 < first + Dh)
                    o_s[(n & 1) * 12 + g, pl.ds(n >> 1, 1), :] = jnp.sum(
                        jnp.where(keep, acc, 0.0), axis=0, keepdims=True)
                return carry

            cells = ns - 4 if last else ns
            wait_all(arena.at[pl.ds(k_block, cells)], n & 1)
            jax.lax.fori_loop(0, 4, scores, 0)
            s = jnp.concatenate([s_s[t] for t in range(4)], axis=1) * scale
            p = jnp.exp(s - jnp.max(s, axis=-1, keepdims=True))
            p_s[...] = (p / jnp.sum(p, axis=-1, keepdims=True)).astype(bf16)
            wait_all(arena.at[pl.ds(v_block, cells)], 2 + (n & 1))
            jax.lax.fori_loop(0, 4, values, 0)

        def period(n, carry):
            attend(n, False)
            return carry

        jax.lax.fori_loop(0, nblk - 1, period, 0)
        attend(nblk - 1, True)

        def w2_piece(m, e, q):
            stage = [2 * n_w2 + m < k for k in _W2_STAGES].index(True)
            pltpu.make_async_copy(w2_hbm.at[m, pl.ds((4 + e) * _MAJ, _MAJ), :],
                                  arena.at[a_w2 + 2 * n_w2 + m, e, :, pl.ds(0, D)],
                                  sem.at[sem_w2 + 1 + stage]).start(priority=q)

        units = [partial(quad_unit, wo_hbm, a_wo, n_wo, sem_wo, u // 4, u % 4)
                 for u in range(HD // 32)]
        w1_units = [partial(strip_unit, w1_hbm, w1_v, 0, sem_w1, m, r, 0, F)
                    for r in range(0, _W1M, 8) for m in range(D // _W1M)]
        w2_units = [partial(quad_unit, w2_hbm, a_w2, n_w2, sem_w2, r, 0) for r in range(32)]
        for r in range(16):
            units += w1_units[5 * r:5 * r + 5] + [w2_units[r]]
        hi = units[0::2]
        lo = units[1::2] + w2_units[16:] + [
            partial(w2_piece, m, e) for m in range(n_w2) for e in range(2)]
        assert len(lo) <= len(hi) + _LAG

        def w_cells(cell, n):
            return arena.at[pl.ds(cell, n), :, :, pl.ds(0, D)]

        s0 = ns + 4 * _NVP
        chunk_step = (s0, s0 + n_wo, HD // 64 + 8)
        attn = jnp.zeros((B, D), f32)
        for t in range(s0, len(hi)):
            if t in chunk_step:
                c3 = chunk_step.index(t)
                wait_all(w_cells(a_wo + n_wo * c3, n_wo), sem_wo + c3)
            hi[t](0)
            if t + _LAG < len(lo):
                lo[t + _LAG](1)
            m = t - chunk_step[c3]
            if m < n_wo:
                col = m * _OM + c3 * 128
                o_t = o_s[col // 256, :, pl.ds(col % 256, 128)].astype(bf16)
                attn = attn + _dot(o_t, w_cells(a_wo + n_wo * c3 + m, 1)[...].reshape(128, D))
            if (c3, m) == (2, n_wo - 1):
                ga, sb, cb, gb = (mod_s[:, k * D:(k + 1) * D] for k in range(2, 6))
                x1 = x + ga * attn
                h2 = _layernorm(x1) * (1.0 + cb) + sb
                y = _layernorm(h2).astype(bf16)

        b1_cp.wait()
        b2_cp.wait()
        wait_all(w1_v, sem_w1)
        u = _dot(y, w1_v[...].reshape(D, F)) + b1_v[...].astype(f32).reshape(1, F)
        u = jax.nn.gelu(u, approximate=True).astype(bf16)

        def w2_dot(k0, k1):
            cols = [k % n_w2 * _OM + k // n_w2 * 128 for k in range(k0, k1)]
            lhs = jnp.concatenate([u[:, j:j + 128] for j in cols], axis=1)
            return _dot(lhs, w_cells(a_w2 + k0, k1 - k0)[...].reshape(128 * (k1 - k0), D))

        for c3 in range(2):
            wait_all(w_cells(a_w2 + n_w2 * c3, n_w2), sem_w2 + c3)
        mlp = b2_v[...].astype(f32).reshape(1, D) + w2_dot(0, _W2_STAGES[0])
        for stage, (k0, k1) in enumerate(zip(_W2_STAGES, _W2_STAGES[1:])):
            wait_all(w_cells(a_w2 + k0, k1 - k0), sem_w2 + 2 + stage)
            mlp = mlp + w2_dot(k0, k1)
        out_ref[...] = (x1 + gb * mlp).astype(out_ref.dtype)

    kv_views = [jnp.swapaxes(a, 2, 3).reshape(nblk * bm // g, g, _MAJ, Sk)
                for a in (A_k_cache, A_v_cache) for g in (2, 6)]

    out = pl.pallas_call(
        kernel,
        out_shape=jax.ShapeDtypeStruct((B, D), A_x.dtype),
        in_specs=[pl.BlockSpec(memory_space=pl.ANY)] * 13,
        out_specs=pl.BlockSpec(memory_space=pltpu.VMEM),
        scratch_shapes=[
            pltpu.VMEM((B, D), bf16),
            pltpu.VMEM((B, D), bf16),
            pltpu.VMEM((F,), bf16),
            pltpu.VMEM((D,), bf16),
            pltpu.VMEM((D // _HM, _HM, HD + 6 * D), bf16),
            pltpu.VMEM((D // _W1M, _W1M, F), bf16),
            pltpu.VMEM((a_end, 2, _MAJ, W), bf16),
            pltpu.VMEM((B, 6 * D), f32),
            pltpu.VMEM((B, D), bf16),
            pltpu.VMEM((W // 256, _HG, 256), f32),
            pltpu.VMEM((_HG, W), bf16),
            pltpu.VMEM((HD // 256, B, 256), f32),
            pltpu.SemaphoreType.DMA((sem_small + 4,)),
        ],
        compiler_params=pltpu.CompilerParams(
            vmem_limit_bytes=100 * 1024 * 1024,
            disable_bounds_checks=True,
            disable_semaphore_checks=True,
        ),
    )(A_x.reshape(B, D), *kv_views, A_wq.reshape(D // _HM, _HM, HD),
      A_wo.reshape(n_wo, _OM, D), B_w1.reshape(D // _W1M, _W1M, F), B_b1,
      B_w2.reshape(n_w2, _OM, D), B_b2, c, w_mod.reshape(D // _HM, _HM, 6 * D))
    return out.reshape(B, Sq, D)
```
